```python
import jax
import jax.numpy as jnp

def _softmax(x, axis=-1):
    return jax.nn.softmax(x, axis=axis)
def _gelu(x):
    return jax.nn.gelu(x, approximate=True)
def _silu(x):
    return jax.nn.silu(x)
def _sigmoid(x):
    return jax.nn.sigmoid(x)
def _layernorm(x, axis=-1, eps=1e-5):
    m = jnp.mean(x, axis=axis, keepdims=True)
    v = jnp.var(x, axis=axis, keepdims=True)
    return (x - m) / jnp.sqrt(v + eps)
def _scatter_add(tgt, idx, src, axis=0):
    return tgt.at[idx].add(src)
def _segment_sum(src, seg, n):
    return jax.ops.segment_sum(src, seg, n)
class _Rng:
    def __init__(self, key):
        self._k = key
    def _next(self):
        self._k, sub = jax.random.split(self._k)
        return sub
    def normal(self, shape):
        return jax.random.normal(self._next(), shape, dtype=jnp.bfloat16)
    def randint(self, lo, hi, shape):
        return jax.random.randint(self._next(), shape, lo, hi, dtype=jnp.int32)
    def uniform(self, shape, lo=0.0, hi=1.0):
        return jax.random.uniform(self._next(), shape, jnp.bfloat16, lo, hi)
    def permutation(self, n):
        return jax.random.permutation(self._next(), n)


kernel_name = 'gated_mix__sliding_block_cached__glu_gated_swiglu__decode'

def setup_inputs():
    _rng = _Rng(jax.random.key(int.from_bytes(__import__("os").urandom(4), "little")))
    _w = (lambda a: (lambda t: t.astype(jnp.bfloat16) if jnp.issubdtype(t.dtype, jnp.floating) else t)(jnp.asarray(a)))
    def _A_setup():
        B, Sq, D = 1, 1, 640
        Hq, Hkv, Sk, Dh = 32, 32, 32768, 192
        assert Hq % Hkv == 0, (Hq, Hkv)
        return {
            "x": _w((lambda *s: _rng.normal(s) * 0.05)(B, Sq, D)),
            "k_cache": _w((lambda *s: _rng.normal(s) * 0.05)(B, Hkv, Sk, Dh)),
            "v_cache": _w((lambda *s: _rng.normal(s) * 0.05)(B, Hkv, Sk, Dh)),
            "wq": _w((lambda *s: _rng.normal(s) * 0.05)(D, Hq * Dh) * (D ** -0.5)),
            "wo": _w((lambda *s: _rng.normal(s) * 0.05)(Hq * Dh, D) * ((Hq * Dh) ** -0.5)),
        }
    _A_in = _A_setup()

    def _B_setup():
        B, S, D, F = 1, 1, 640, 1536
        return {
            "x": _w((lambda *s: _rng.normal(s) * 0.05)(B, S, D)),
            "w1": _w((lambda *s: _rng.normal(s) * 0.05)(D, F) * (2.0 / D) ** 0.5),
            "w3": _w((lambda *s: _rng.normal(s) * 0.05)(D, F) * (2.0 / D) ** 0.5),
            "w2": _w((lambda *s: _rng.normal(s) * 0.05)(F, D) * (2.0 / F) ** 0.5),
        }
    _B_in = _B_setup()

    return {
        "A_x": _A_in["x"],
        "A_k_cache": _A_in["k_cache"],
        "A_v_cache": _A_in["v_cache"],
        "A_wq": _A_in["wq"],
        "A_wo": _A_in["wo"],
        "B_x": _B_in["x"],
        "B_w1": _B_in["w1"],
        "B_w3": _B_in["w3"],
        "B_w2": _B_in["w2"],
        "gate_w": _w((lambda *s: _rng.normal(s) * 0.05)(640)),
    }

def reference(A_x, A_k_cache, A_v_cache, A_wq, A_wo, B_x, B_w1, B_w3, B_w2, gate_w):
    def _A_ref(x, k_cache, v_cache, wq, wo):
        B, Sq, D = x.shape
        Hq, Dh = 32, 192
        Hkv, Sk = k_cache.shape[1], k_cache.shape[2]
        W = min(4096, max(256, Sk // 4))
        rep = Hq // Hkv
        q = (lambda x, *d: x.transpose(*d))((x @ wq).reshape(B, Sq, Hq, Dh), 0, 2, 1, 3)
        k = jnp.repeat(k_cache[:, :, Sk - W:, :], rep, axis=1)
        v = jnp.repeat(v_cache[:, :, Sk - W:, :], rep, axis=1)
        scores = jnp.einsum("bhqd,bhkd->bhqk", q, k) * (Dh ** -0.5)
        p = _softmax(scores, axis=-1)
        o = jnp.einsum("bhqk,bhkd->bhqd", p, v)
        return (lambda x, *d: x.transpose(*d))(o, 0, 2, 1, 3).reshape(B, Sq, Hq * Dh) @ wo

    def _B_ref(x, w1, w3, w2):
        gate = jnp.einsum("bsd,df->bsf", x, w1)
        up = jnp.einsum("bsd,df->bsf", x, w3)
        h = _silu(gate) * up
        out = jnp.einsum("bsf,fd->bsd", h, w2)
        return out

    x = A_x
    g = _sigmoid((x * gate_w).sum(-1, keepdims=True))
    a = _A_ref(x, A_k_cache, A_v_cache, A_wq, A_wo)
    b = _B_ref(x, B_w1, B_w3, B_w2)
    return g * a + (1 - g) * b
```

```python
import functools

import jax
import jax.numpy as jnp
from jax import lax
import jax.experimental.pallas as pl
import jax.experimental.pallas.tpu as pltpu

D = 640
HQ = 32
DH = 192
HD = HQ * DH
F = 1536
G = 2
GR = G * DH
NG = HQ // G
NB = 4
LROWS = 8

_NT = (((1,), (1,)), ((), ()))


def _kernel(x_hbm, gw_hbm, k_hbm, v_hbm, wq_hbm, wo_hbm, w1_hbm, w3_hbm, w2_hbm,
            o_ref,
            x_v, gw_v, wq_v, wo_v, w1_v, w3_v, w2_v, kv_v, q_s, r_s,
            sem_w, sem_kv, sem_wo, *, sk, win):
  col0 = sk - win
  scale = DH ** -0.5

  def kv_copy(i, slot):
    g = i // 2
    rows = pl.ds(pl.multiple_of(g * GR, GR), GR)
    return (pltpu.make_async_copy(k_hbm.at[rows, pl.ds(col0, win)], kv_v.at[slot], sem_kv.at[slot]),
            pltpu.make_async_copy(v_hbm.at[rows, pl.ds(col0, win)], kv_v.at[slot], sem_kv.at[slot]))

  def k_copy(g, slot):
    rows = pl.ds(g * GR, GR) if isinstance(g, int) else pl.ds(pl.multiple_of(g * GR, GR), GR)
    return pltpu.make_async_copy(k_hbm.at[rows, pl.ds(col0, win)], kv_v.at[slot], sem_kv.at[slot])

  def v_copy(g, slot):
    rows = pl.ds(g * GR, GR) if isinstance(g, int) else pl.ds(pl.multiple_of(g * GR, GR), GR)
    return pltpu.make_async_copy(v_hbm.at[rows, pl.ds(col0, win)], kv_v.at[slot], sem_kv.at[slot])

  def wo_copy(c):
    rows = pl.ds(c * GR, GR) if isinstance(c, int) else pl.ds(pl.multiple_of(c * GR, GR), GR)
    return pltpu.make_async_copy(wo_hbm.at[rows, :], wo_v.at[rows, :], sem_wo.at[c])

  cp_wq = pltpu.make_async_copy(wq_hbm, wq_v, sem_w.at[0])
  cp_x = pltpu.make_async_copy(x_hbm, x_v, sem_w.at[1])
  cp_gw = pltpu.make_async_copy(gw_hbm, gw_v, sem_w.at[2])
  cp_w1 = pltpu.make_async_copy(w1_hbm, w1_v, sem_w.at[3])
  cp_w3 = pltpu.make_async_copy(w3_hbm, w3_v, sem_w.at[4])
  cp_w2 = pltpu.make_async_copy(w2_hbm, w2_v, sem_w.at[5])

  cp_wq.start()
  cp_x.start()
  cp_gw.start()
  k_copy(0, 0).start()
  v_copy(0, 1).start()
  cp_w1.start()
  cp_w3.start()

  cp_x.wait()
  cp_gw.wait()
  x = x_v[...]
  x8 = jnp.broadcast_to(x, (LROWS, D))
  gate_logit = jnp.sum(x.astype(jnp.float32) * gw_v[...].astype(jnp.float32),
                       axis=-1, keepdims=True)
  gmix = jax.nn.sigmoid(gate_logit)

  row = lax.broadcasted_iota(jnp.int32, (LROWS, GR), 0)
  head_in_group = lax.broadcasted_iota(jnp.int32, (LROWS, GR), 1) // DH
  diag = row == head_in_group

  cp_wq.wait()
  for g in range(NG):
    qg = jnp.dot(x8, wq_v[:, g * GR:(g + 1) * GR], preferred_element_type=jnp.float32)
    q_s[g] = jnp.where(diag, qg.astype(jnp.bfloat16).astype(jnp.float32), 0.0)

  for s in range(2, NB):
    if s % 2 == 0:
      k_copy(s // 2, s).start()
    else:
      v_copy(s // 2, s).start()

  cp_w1.wait()
  cp_w3.wait()
  gate = jnp.dot(x8, w1_v[...], preferred_element_type=jnp.float32)
  up = jnp.dot(x8, w3_v[...], preferred_element_type=jnp.float32)
  gate = gate.astype(jnp.bfloat16).astype(jnp.float32)
  up = up.astype(jnp.bfloat16).astype(jnp.float32)
  h8 = (gate * jax.nn.sigmoid(gate) * up).astype(jnp.bfloat16)

  assert NB % 2 == 0
  GA = NB // 2

  def group(g, carry):
    ks = lax.rem(2 * g, NB)
    vs = ks + 1
    qb = q_s[g].astype(jnp.bfloat16)
    k_copy(g, ks).wait()
    s = jnp.dot(qb, kv_v[ks], preferred_element_type=jnp.float32) * scale
    m = jnp.max(s, axis=-1, keepdims=True)
    e = jnp.exp(s - m)
    l = jnp.sum(e, axis=-1, keepdims=True)
    p = e.astype(jnp.bfloat16)

    @pl.when(g + GA < NG)
    def _():
      k_copy(g + GA, ks).start()

    v_copy(g, vs).wait()
    r = lax.dot_general(p, kv_v[vs], _NT, preferred_element_type=jnp.float32)
    r_s[g] = jnp.where(diag, r / l, 0.0)

    @pl.when(g + GA < NG)
    def _():
      v_copy(g + GA, vs).start()

    @pl.when(g + GA == NG)
    def _():
      cp_w2.start()
      for c in range(NG):
        wo_copy(c).start()
    return carry

  lax.fori_loop(0, NG, group, 0)

  cp_w2.wait()
  b8 = jnp.dot(h8, w2_v[...], preferred_element_type=jnp.float32)

  def out_chunk(c, acc):
    wo_copy(c).wait()
    rows = pl.ds(pl.multiple_of(c * GR, GR), GR)
    return acc + jnp.dot(r_s[c].astype(jnp.bfloat16), wo_v[rows, :],
                         preferred_element_type=jnp.float32)

  acc = lax.fori_loop(0, NG, out_chunk, jnp.zeros((LROWS, D), jnp.float32))
  a = jnp.sum(acc, axis=0, keepdims=True)
  b = b8[0:1, :]
  o_ref[...] = (gmix * a + (1.0 - gmix) * b).astype(o_ref.dtype)


@jax.jit
def pallas_gated_mix__sliding_block_cached__glu_gated_swiglu__decode_kernel(
    A_x: jax.Array,
    A_k_cache: jax.Array,
    A_v_cache: jax.Array,
    A_wq: jax.Array,
    A_wo: jax.Array,
    B_x: jax.Array,
    B_w1: jax.Array,
    B_w3: jax.Array,
    B_w2: jax.Array,
    gate_w: jax.Array,
):
  del B_x
  sk = A_k_cache.shape[2]
  win = min(4096, max(256, sk // 4))
  assert A_k_cache.shape == (1, HQ, sk, DH) and A_x.shape == (1, 1, D)

  kt = jnp.swapaxes(A_k_cache, 2, 3).reshape(HD, sk)
  vt = jnp.swapaxes(A_v_cache, 2, 3).reshape(HD, sk)

  any_spec = pl.BlockSpec(memory_space=pl.ANY)
  bf16 = jnp.bfloat16
  out = pl.pallas_call(
      functools.partial(_kernel, sk=sk, win=win),
      out_shape=jax.ShapeDtypeStruct((1, D), A_x.dtype),
      in_specs=[any_spec] * 9,
      out_specs=pl.BlockSpec(memory_space=pltpu.VMEM),
      scratch_shapes=[
          pltpu.VMEM((1, D), bf16),
          pltpu.VMEM((1, D), bf16),
          pltpu.VMEM((D, HD), bf16),
          pltpu.VMEM((HD, D), bf16),
          pltpu.VMEM((D, F), bf16),
          pltpu.VMEM((D, F), bf16),
          pltpu.VMEM((F, D), bf16),
          pltpu.VMEM((NB, GR, win), bf16),
          pltpu.VMEM((NG, LROWS, GR), jnp.float32),
          pltpu.VMEM((NG, LROWS, GR), jnp.float32),
          pltpu.SemaphoreType.DMA((6,)),
          pltpu.SemaphoreType.DMA((NB,)),
          pltpu.SemaphoreType.DMA((NG,)),
      ],
      compiler_params=pltpu.CompilerParams(vmem_limit_bytes=100 * 1024 * 1024),
  )(A_x.reshape(1, D), gate_w.reshape(1, D), kt, vt, A_wq, A_wo, B_w1, B_w3, B_w2)
  return out.reshape(1, 1, D)
```

```python
import functools

import jax
import jax.numpy as jnp
from jax import lax
import jax.experimental.pallas as pl
import jax.experimental.pallas.tpu as pltpu

D = 640
HQ = 32
DH = 192
HD = HQ * DH
F = 1536
G = 2
GR = G * DH
NG = HQ // G
GA = 2
NB = 2 * GA
LROWS = 8
W2_SPLITS = (1408, 128)
GW_MODE = "5x128"

_NT = (((1,), (1,)), ((), ()))


def _kernel(x_hbm, gw_hbm, k_hbm, v_hbm, wq_hbm, wo_hbm, w1_hbm, w3_hbm, w2_hbm,
            o_ref,
            x_v, gw_v, wq_v, wo_v, w1_v, w3_v, w2_v, kv_v, q_s,
            sem_a, sem_kv, sem_wo, *, sk, win):
  col0 = sk - win
  scale = DH ** -0.5

  def rows_of(g):
    return pl.ds(g * GR, GR) if isinstance(g, int) else pl.ds(pl.multiple_of(g * GR, GR), GR)

  def k_copy(g, slot):
    return pltpu.make_async_copy(k_hbm.at[rows_of(g), pl.ds(col0, win)], kv_v.at[slot], sem_kv.at[slot])

  def v_copy(g, slot):
    return pltpu.make_async_copy(v_hbm.at[rows_of(g), pl.ds(col0, win)], kv_v.at[slot], sem_kv.at[slot])

  def wo_copy(g, slot):
    return pltpu.make_async_copy(wo_hbm.at[rows_of(g), :], wo_v.at[slot], sem_wo.at[slot])

  cp_wq = pltpu.make_async_copy(wq_hbm, wq_v, sem_a.at[0])
  cp_x = pltpu.make_async_copy(x_hbm, x_v, sem_a.at[0])
  cp_gw = pltpu.make_async_copy(gw_hbm, gw_v, sem_a.at[0])
  cp_w1 = pltpu.make_async_copy(w1_hbm, w1_v, sem_a.at[1])
  cp_w3 = pltpu.make_async_copy(w3_hbm, w3_v, sem_a.at[1])
  w2_offs = [sum(W2_SPLITS[:i]) for i in range(len(W2_SPLITS))]
  assert sum(W2_SPLITS) == F and len(W2_SPLITS) <= 2
  cp_w2 = [pltpu.make_async_copy(w2_hbm.at[pl.ds(o, n), :], w2_v.at[pl.ds(o, n), :], sem_a.at[i])
           for i, (o, n) in enumerate(zip(w2_offs, W2_SPLITS))]

  cp_wq.start()
  cp_x.start()
  cp_gw.start()
  for g in range(GA):
    k_copy(g, 2 * g).start()
    v_copy(g, 2 * g + 1).start()
    wo_copy(g, g).start()
    if g == 0:
      cp_w1.start()
      cp_w3.start()

  cp_wq.wait()
  cp_x.wait()
  cp_gw.wait()
  x = x_v[...]
  x8 = jnp.broadcast_to(x, (LROWS, D))
  xf = x.astype(jnp.float32)
  if GW_MODE == "5x128":
    gwf = gw_v[...].astype(jnp.float32)
    prod = xf[:, 0:128] * gwf[0:1, :]
    for r in range(1, D // 128):
      prod = prod + xf[:, r * 128:(r + 1) * 128] * gwf[r:r + 1, :]
    gate_logit = jnp.sum(prod, axis=-1, keepdims=True)
  elif GW_MODE == "1d":
    gate_logit = jnp.sum(xf * gw_v[...].astype(jnp.float32).reshape(1, D), axis=-1, keepdims=True)
  else:
    gate_logit = jnp.sum(xf * gw_v[...].astype(jnp.float32), axis=-1, keepdims=True)
  gmix = jax.nn.sigmoid(gate_logit)

  row = lax.broadcasted_iota(jnp.int32, (LROWS, GR), 0)
  head_in_group = lax.broadcasted_iota(jnp.int32, (LROWS, GR), 1) // DH
  diag = row == head_in_group

  for g in range(NG):
    qg = jnp.dot(x8, wq_v[:, g * GR:(g + 1) * GR], preferred_element_type=jnp.float32)
    q_s[g] = jnp.where(diag, qg.astype(jnp.bfloat16).astype(jnp.float32), 0.0)

  cp_w1.wait()
  cp_w3.wait()
  gate = jnp.dot(x8, w1_v[...], preferred_element_type=jnp.float32)
  up = jnp.dot(x8, w3_v[...], preferred_element_type=jnp.float32)
  gate = gate.astype(jnp.bfloat16).astype(jnp.float32)
  up = up.astype(jnp.bfloat16).astype(jnp.float32)
  h8 = (gate * jax.nn.sigmoid(gate) * up).astype(jnp.bfloat16)

  def group(g, acc):
    ks = 2 * lax.rem(g, GA)
    vs = ks + 1
    ws = lax.rem(g, GA)
    more = g + GA < NG
    qb = q_s[g].astype(jnp.bfloat16)
    k_copy(g, ks).wait()
    s = jnp.dot(qb, kv_v[ks], preferred_element_type=jnp.float32) * scale

    @pl.when(more)
    def _():
      k_copy(g + GA, ks).start()

    @pl.when(g + GA == NG)
    def _():
      for cp in cp_w2:
        cp.start()

    m = jnp.max(s, axis=-1, keepdims=True)
    e = jnp.exp(s - m)
    l = jnp.sum(e, axis=-1, keepdims=True)
    p = e.astype(jnp.bfloat16)

    v_copy(g, vs).wait()
    r = lax.dot_general(p, kv_v[vs], _NT, preferred_element_type=jnp.float32)

    @pl.when(more)
    def _():
      v_copy(g + GA, vs).start()

    o = jnp.where(diag, r / l, 0.0).astype(jnp.bfloat16)
    wo_copy(g, ws).wait()
    acc = acc + jnp.dot(o, wo_v[ws], preferred_element_type=jnp.float32)

    @pl.when(more)
    def _():
      wo_copy(g + GA, ws).start()
    return acc

  acc = lax.fori_loop(0, NG, group, jnp.zeros((LROWS, D), jnp.float32))

  out = gmix * jnp.sum(acc, axis=0, keepdims=True)
  b = None
  for cp, o_, n in zip(cp_w2, w2_offs, W2_SPLITS):
    cp.wait()
    part = jnp.dot(h8[:, o_:o_ + n], w2_v[pl.ds(o_, n), :], preferred_element_type=jnp.float32)
    b = part if b is None else b + part
  o_ref[...] = (out + (1.0 - gmix) * b[0:1, :]).astype(o_ref.dtype)


@jax.jit
def pallas_gated_mix__sliding_block_cached__glu_gated_swiglu__decode_kernel(
    A_x, A_k_cache, A_v_cache, A_wq, A_wo, B_x, B_w1, B_w3, B_w2, gate_w):
  del B_x
  sk = A_k_cache.shape[2]
  win = min(4096, max(256, sk // 4))
  assert A_k_cache.shape == (1, HQ, sk, DH) and A_x.shape == (1, 1, D)
  kt = jnp.swapaxes(A_k_cache, 2, 3).reshape(HD, sk)
  vt = jnp.swapaxes(A_v_cache, 2, 3).reshape(HD, sk)
  gw_shape = {"5x128": (D // 128, 128), "1d": (D,), "2d": (1, D)}[GW_MODE]
  any_spec = pl.BlockSpec(memory_space=pl.ANY)
  bf16 = jnp.bfloat16
  out = pl.pallas_call(
      functools.partial(_kernel, sk=sk, win=win),
      out_shape=jax.ShapeDtypeStruct((1, D), A_x.dtype),
      in_specs=[any_spec] * 9,
      out_specs=pl.BlockSpec(memory_space=pltpu.VMEM),
      scratch_shapes=[
          pltpu.VMEM((1, D), bf16),
          pltpu.VMEM(gw_shape, bf16),
          pltpu.VMEM((D, HD), bf16),
          pltpu.VMEM((GA, GR, D), bf16),
          pltpu.VMEM((D, F), bf16),
          pltpu.VMEM((D, F), bf16),
          pltpu.VMEM((F, D), bf16),
          pltpu.VMEM((NB, GR, win), bf16),
          pltpu.VMEM((NG, LROWS, GR), jnp.float32),
          pltpu.SemaphoreType.DMA((2,)),
          pltpu.SemaphoreType.DMA((NB,)),
          pltpu.SemaphoreType.DMA((GA,)),
      ],
      compiler_params=pltpu.CompilerParams(vmem_limit_bytes=100 * 1024 * 1024),
  )(A_x.reshape(1, D), gate_w.reshape(gw_shape), kt, vt, A_wq, A_wo, B_w1, B_w3, B_w2)
  return out.reshape(1, 1, D)
```

```python
import functools

import jax
import jax.numpy as jnp
from jax import lax
import jax.experimental.pallas as pl
import jax.experimental.pallas.tpu as pltpu

D = 640
HQ = 32
DH = 192
HD = HQ * DH
F = 1536
G = 2
GR = G * DH
NG = HQ // G
GA = 2
NB = 2 * GA
LROWS = 8
W2_SPLITS = (1408, 128)
GW_MODE = "5x128"

_NT = (((1,), (1,)), ((), ()))


def _kernel(x_hbm, gw_hbm, k_hbm, v_hbm, wq_hbm, wo_hbm, w1_hbm, w3_hbm, w2_hbm,
            o_ref,
            x_v, gw_v, wq_v, wo_v, w1_v, w3_v, w2_v, kv_v, q_s, base_s,
            sem_a, sem_kv, sem_wo, *, sk, win):
  col0 = sk - win
  scale = DH ** -0.5

  def rows_of(g):
    return pl.ds(g * GR, GR) if isinstance(g, int) else pl.ds(pl.multiple_of(g * GR, GR), GR)

  def k_copy(g, slot):
    return pltpu.make_async_copy(k_hbm.at[rows_of(g), pl.ds(col0, win)], kv_v.at[slot], sem_kv.at[slot])

  def v_copy(g, slot):
    return pltpu.make_async_copy(v_hbm.at[rows_of(g), pl.ds(col0, win)], kv_v.at[slot], sem_kv.at[slot])

  def wo_copy(g, slot):
    return pltpu.make_async_copy(wo_hbm.at[rows_of(g), :], wo_v.at[slot], sem_wo.at[slot])

  cp_wq = pltpu.make_async_copy(wq_hbm, wq_v, sem_a.at[0])
  cp_x = pltpu.make_async_copy(x_hbm, x_v, sem_a.at[0])
  cp_gw = pltpu.make_async_copy(gw_hbm, gw_v, sem_a.at[0])
  cp_w1 = pltpu.make_async_copy(w1_hbm, w1_v, sem_a.at[1])
  cp_w3 = pltpu.make_async_copy(w3_hbm, w3_v, sem_a.at[1])
  w2_offs = [sum(W2_SPLITS[:i]) for i in range(len(W2_SPLITS))]
  assert sum(W2_SPLITS) == F and len(W2_SPLITS) <= 2
  cp_w2 = [pltpu.make_async_copy(w2_hbm.at[pl.ds(o, n), :], w2_v.at[pl.ds(o, n), :], sem_a.at[i])
           for i, (o, n) in enumerate(zip(w2_offs, W2_SPLITS))]

  cp_wq.start()
  cp_x.start()
  cp_gw.start()
  for g in range(GA):
    k_copy(g, 2 * g).start()
    v_copy(g, 2 * g + 1).start()
    wo_copy(g, g).start()
    if g == 0:
      cp_w1.start()
      cp_w3.start()

  cp_wq.wait()
  cp_x.wait()
  cp_gw.wait()
  x = x_v[...]
  x8 = jnp.broadcast_to(x, (LROWS, D))
  xf = x.astype(jnp.float32)
  if GW_MODE == "5x128":
    gwf = gw_v[...].astype(jnp.float32)
    prod = xf[:, 0:128] * gwf[0:1, :]
    for r in range(1, D // 128):
      prod = prod + xf[:, r * 128:(r + 1) * 128] * gwf[r:r + 1, :]
    gate_logit = jnp.sum(prod, axis=-1, keepdims=True)
  elif GW_MODE == "1d":
    gate_logit = jnp.sum(xf * gw_v[...].astype(jnp.float32).reshape(1, D), axis=-1, keepdims=True)
  else:
    gate_logit = jnp.sum(xf * gw_v[...].astype(jnp.float32), axis=-1, keepdims=True)
  gmix = jax.nn.sigmoid(gate_logit)

  row = lax.broadcasted_iota(jnp.int32, (LROWS, GR), 0)
  head_in_group = lax.broadcasted_iota(jnp.int32, (LROWS, GR), 1) // DH
  diag = row == head_in_group

  for g in range(NG):
    qg = jnp.dot(x8, wq_v[:, g * GR:(g + 1) * GR], preferred_element_type=jnp.float32)
    q_s[g] = jnp.where(diag, qg.astype(jnp.bfloat16).astype(jnp.float32), 0.0)

  cp_w1.wait()
  cp_w3.wait()
  gate = jnp.dot(x8, w1_v[...], preferred_element_type=jnp.float32)
  up = jnp.dot(x8, w3_v[...], preferred_element_type=jnp.float32)
  gate = gate.astype(jnp.bfloat16).astype(jnp.float32)
  up = up.astype(jnp.bfloat16).astype(jnp.float32)
  h8 = (gate * jax.nn.sigmoid(gate) * up).astype(jnp.bfloat16)

  def group(g, acc):
    ks = 2 * lax.rem(g, GA)
    vs = ks + 1
    ws = lax.rem(g, GA)
    more = g + GA < NG
    qb = q_s[g].astype(jnp.bfloat16)
    k_copy(g, ks).wait()
    s = jnp.dot(qb, kv_v[ks], preferred_element_type=jnp.float32) * scale

    @pl.when(more)
    def _():
      k_copy(g + GA, ks).start()

    @pl.when(g + GA == NG)
    def _():
      for cp in cp_w2:
        cp.start()

    m = jnp.max(s, axis=-1, keepdims=True)
    e = jnp.exp(s - m)
    l = jnp.sum(e, axis=-1, keepdims=True)
    p = e.astype(jnp.bfloat16)

    v_copy(g, vs).wait()
    r = lax.dot_general(p, kv_v[vs], _NT, preferred_element_type=jnp.float32)

    @pl.when(more)
    def _():
      v_copy(g + GA, vs).start()

    o = jnp.where(diag, r / l, 0.0).astype(jnp.bfloat16)
    wo_copy(g, ws).wait()
    acc = acc + jnp.dot(o, wo_v[ws], preferred_element_type=jnp.float32)

    @pl.when(more)
    def _():
      wo_copy(g + GA, ws).start()
    return acc

  acc = lax.fori_loop(0, NG, group, jnp.zeros((LROWS, D), jnp.float32))

  out = gmix * jnp.sum(acc, axis=0, keepdims=True)
  for i, (cp, o_, n) in enumerate(zip(cp_w2, w2_offs, W2_SPLITS)):
    if i > 0:
      out = base_s[...]
    cp.wait()
    part = jnp.dot(h8[:, o_:o_ + n], w2_v[pl.ds(o_, n), :], preferred_element_type=jnp.float32)
    out = out + (1.0 - gmix) * part[0:1, :]
    if i + 1 < len(cp_w2):
      base_s[...] = out
  o_ref[...] = out.astype(o_ref.dtype)


@jax.jit
def pallas_gated_mix__sliding_block_cached__glu_gated_swiglu__decode_kernel(
    A_x, A_k_cache, A_v_cache, A_wq, A_wo, B_x, B_w1, B_w3, B_w2, gate_w):
  del B_x
  sk = A_k_cache.shape[2]
  win = min(4096, max(256, sk // 4))
  assert A_k_cache.shape == (1, HQ, sk, DH) and A_x.shape == (1, 1, D)
  kt = jnp.swapaxes(A_k_cache, 2, 3).reshape(HD, sk)
  vt = jnp.swapaxes(A_v_cache, 2, 3).reshape(HD, sk)
  gw_shape = {"5x128": (D // 128, 128), "1d": (D,), "2d": (1, D)}[GW_MODE]
  any_spec = pl.BlockSpec(memory_space=pl.ANY)
  bf16 = jnp.bfloat16
  out = pl.pallas_call(
      functools.partial(_kernel, sk=sk, win=win),
      out_shape=jax.ShapeDtypeStruct((1, D), A_x.dtype),
      in_specs=[any_spec] * 9,
      out_specs=pl.BlockSpec(memory_space=pltpu.VMEM),
      scratch_shapes=[
          pltpu.VMEM((1, D), bf16),
          pltpu.VMEM(gw_shape, bf16),
          pltpu.VMEM((D, HD), bf16),
          pltpu.VMEM((GA, GR, D), bf16),
          pltpu.VMEM((D, F), bf16),
          pltpu.VMEM((D, F), bf16),
          pltpu.VMEM((F, D), bf16),
          pltpu.VMEM((NB, GR, win), bf16),
          pltpu.VMEM((NG, LROWS, GR), jnp.float32),
          pltpu.VMEM((1, D), jnp.float32),
          pltpu.SemaphoreType.DMA((2,)),
          pltpu.SemaphoreType.DMA((NB,)),
          pltpu.SemaphoreType.DMA((GA,)),
      ],
      compiler_params=pltpu.CompilerParams(vmem_limit_bytes=100 * 1024 * 1024),
  )(A_x.reshape(1, D), gate_w.reshape(gw_shape), kt, vt, A_wq, A_wo, B_w1, B_w3, B_w2)
  return out.reshape(1, 1, D)
```

```python
import functools

import jax
import jax.numpy as jnp
from jax import lax
import jax.experimental.pallas as pl
import jax.experimental.pallas.tpu as pltpu

D = 640
HQ = 32
DH = 192
HD = HQ * DH
F = 1536
G = 2
GR = G * DH
NG = HQ // G
GA = 2
NB = 2 * GA
LROWS = 8
W2_SPLITS = (1024, 384, 128)
KV_CUT = (96, 128, (0, 0, 1, 1), "r")
WQ_CUT = (128, 128, (0, 1), "r")
WO_CUT = (128, 128, (0, 1), "r")
W13_CUT = (128, 128, (0, 1), "r")
W2_CUT = (128, 128, (0, 1), "r")

_NT = (((1,), (1,)), ((), ()))


def _start_cut(src, dst, sem, cut):
  sr, sc, pat, order = cut
  rows, cols = dst.shape
  sr, sc = min(sr, rows), min(sc, cols)
  assert rows % sr == 0 and cols % sc == 0, (dst.shape, cut)
  if order == "r":
    subs = [(r, c) for r in range(0, rows, sr) for c in range(0, cols, sc)]
  else:
    subs = [(r, c) for c in range(0, cols, sc) for r in range(0, rows, sr)]
  for j, (r, c) in enumerate(subs):
    pltpu.make_async_copy(src.at[pl.ds(r, sr), pl.ds(c, sc)], dst.at[pl.ds(r, sr), pl.ds(c, sc)],
                          sem).start(priority=pat[j % len(pat)])


def _wait_all(dst, sem):
  pltpu.make_async_copy(dst, dst, sem).wait()


def _kernel(x_hbm, gw_hbm, k_hbm, v_hbm, wq_hbm, wo_hbm, w1_hbm, w3_hbm, w2_hbm,
            o_ref,
            x_v, gw_v, wq_v, wo_v, w1_v, w3_v, w2_v, kv_v, q_s, base_s,
            sem_a, sem_kv, sem_wo, *, sk, win):
  col0 = sk - win
  scale = DH ** -0.5

  def rows_of(g):
    return pl.ds(g * GR, GR) if isinstance(g, int) else pl.ds(pl.multiple_of(g * GR, GR), GR)

  def k_start(g, slot):
    _start_cut(k_hbm.at[rows_of(g), pl.ds(col0, win)], kv_v.at[slot], sem_kv.at[slot], KV_CUT)

  def v_start(g, slot):
    _start_cut(v_hbm.at[rows_of(g), pl.ds(col0, win)], kv_v.at[slot], sem_kv.at[slot], KV_CUT)

  def wo_start(g, slot):
    _start_cut(wo_hbm.at[rows_of(g), :], wo_v.at[slot], sem_wo.at[slot], WO_CUT)

  cp_x = pltpu.make_async_copy(x_hbm, x_v, sem_a.at[0])
  cp_gw = pltpu.make_async_copy(gw_hbm, gw_v, sem_a.at[0])
  w2_offs = [sum(W2_SPLITS[:i]) for i in range(len(W2_SPLITS))]
  assert sum(W2_SPLITS) == F and len(W2_SPLITS) <= 3
  w2_sems = [sem_a.at[0], sem_a.at[1], sem_kv.at[2 * ((NG - GA) % GA)]]
  w2_dst = [w2_v.at[pl.ds(o, n), :] for o, n in zip(w2_offs, W2_SPLITS)]
  w2_src = [w2_hbm.at[pl.ds(o, n), :] for o, n in zip(w2_offs, W2_SPLITS)]

  _start_cut(wq_hbm, wq_v, sem_a.at[0], WQ_CUT)
  cp_x.start()
  cp_gw.start()
  for g in range(GA):
    k_start(g, 2 * g)
    v_start(g, 2 * g + 1)
    wo_start(g, g)
    if g == 0:
      _start_cut(w1_hbm, w1_v, sem_a.at[1], W13_CUT)
      _start_cut(w3_hbm, w3_v, sem_a.at[1], W13_CUT)

  _wait_all(wq_v, sem_a.at[0])
  cp_x.wait()
  cp_gw.wait()
  x = x_v[...]
  x8 = jnp.broadcast_to(x, (LROWS, D))
  xf = x.astype(jnp.float32)
  gwf = gw_v[...].astype(jnp.float32)
  prod = xf[:, 0:128] * gwf[0:1, :]
  for r in range(1, D // 128):
    prod = prod + xf[:, r * 128:(r + 1) * 128] * gwf[r:r + 1, :]
  gate_logit = jnp.sum(prod, axis=-1, keepdims=True)
  gmix = jax.nn.sigmoid(gate_logit)

  row = lax.broadcasted_iota(jnp.int32, (LROWS, GR), 0)
  head_in_group = lax.broadcasted_iota(jnp.int32, (LROWS, GR), 1) // DH
  diag = row == head_in_group

  for g in range(NG):
    qg = jnp.dot(x8, wq_v[:, g * GR:(g + 1) * GR], preferred_element_type=jnp.float32)
    q_s[g] = jnp.where(diag, qg.astype(jnp.bfloat16).astype(jnp.float32), 0.0)

  _wait_all(w1_v, sem_a.at[1])
  _wait_all(w3_v, sem_a.at[1])
  gate = jnp.dot(x8, w1_v[...], preferred_element_type=jnp.float32)
  up = jnp.dot(x8, w3_v[...], preferred_element_type=jnp.float32)
  gate = gate.astype(jnp.bfloat16).astype(jnp.float32)
  up = up.astype(jnp.bfloat16).astype(jnp.float32)
  h8 = (gate * jax.nn.sigmoid(gate) * up).astype(jnp.bfloat16)

  def group(g, acc):
    ks = 2 * lax.rem(g, GA)
    vs = ks + 1
    ws = lax.rem(g, GA)
    more = g + GA < NG
    qb = q_s[g].astype(jnp.bfloat16)
    _wait_all(kv_v.at[ks], sem_kv.at[ks])
    s = jnp.dot(qb, kv_v[ks], preferred_element_type=jnp.float32) * scale

    @pl.when(more)
    def _():
      k_start(g + GA, ks)

    @pl.when(g + GA == NG)
    def _():
      for src, dst, sem in zip(w2_src, w2_dst, w2_sems):
        _start_cut(src, dst, sem, W2_CUT)

    m = jnp.max(s, axis=-1, keepdims=True)
    e = jnp.exp(s - m)
    l = jnp.sum(e, axis=-1, keepdims=True)
    p = e.astype(jnp.bfloat16)

    _wait_all(kv_v.at[vs], sem_kv.at[vs])
    r = lax.dot_general(p, kv_v[vs], _NT, preferred_element_type=jnp.float32)

    @pl.when(more)
    def _():
      v_start(g + GA, vs)

    o = jnp.where(diag, r / l, 0.0).astype(jnp.bfloat16)
    _wait_all(wo_v.at[ws], sem_wo.at[ws])
    acc = acc + jnp.dot(o, wo_v[ws], preferred_element_type=jnp.float32)

    @pl.when(more)
    def _():
      wo_start(g + GA, ws)
    return acc

  acc = lax.fori_loop(0, NG, group, jnp.zeros((LROWS, D), jnp.float32))

  out = gmix * jnp.sum(acc, axis=0, keepdims=True)
  for i, (o_, n) in enumerate(zip(w2_offs, W2_SPLITS)):
    if i > 0:
      out = base_s[...]
    _wait_all(w2_dst[i], w2_sems[i])
    part = jnp.dot(h8[:, o_:o_ + n], w2_v[pl.ds(o_, n), :], preferred_element_type=jnp.float32)
    out = out + (1.0 - gmix) * part[0:1, :]
    if i + 1 < len(W2_SPLITS):
      base_s[...] = out
  o_ref[...] = out.astype(o_ref.dtype)


@jax.jit
def pallas_gated_mix__sliding_block_cached__glu_gated_swiglu__decode_kernel(
    A_x, A_k_cache, A_v_cache, A_wq, A_wo, B_x, B_w1, B_w3, B_w2, gate_w):
  del B_x
  sk = A_k_cache.shape[2]
  win = min(4096, max(256, sk // 4))
  assert A_k_cache.shape == (1, HQ, sk, DH) and A_x.shape == (1, 1, D)
  kt = jnp.swapaxes(A_k_cache, 2, 3).reshape(HD, sk)
  vt = jnp.swapaxes(A_v_cache, 2, 3).reshape(HD, sk)
  any_spec = pl.BlockSpec(memory_space=pl.ANY)
  bf16 = jnp.bfloat16
  out = pl.pallas_call(
      functools.partial(_kernel, sk=sk, win=win),
      out_shape=jax.ShapeDtypeStruct((1, D), A_x.dtype),
      in_specs=[any_spec] * 9,
      out_specs=pl.BlockSpec(memory_space=pltpu.VMEM),
      scratch_shapes=[
          pltpu.VMEM((1, D), bf16),
          pltpu.VMEM((D // 128, 128), bf16),
          pltpu.VMEM((D, HD), bf16),
          pltpu.VMEM((GA, GR, D), bf16),
          pltpu.VMEM((D, F), bf16),
          pltpu.VMEM((D, F), bf16),
          pltpu.VMEM((F, D), bf16),
          pltpu.VMEM((NB, GR, win), bf16),
          pltpu.VMEM((NG, LROWS, GR), jnp.float32),
          pltpu.VMEM((1, D), jnp.float32),
          pltpu.SemaphoreType.DMA((2,)),
          pltpu.SemaphoreType.DMA((NB,)),
          pltpu.SemaphoreType.DMA((GA,)),
      ],
      compiler_params=pltpu.CompilerParams(vmem_limit_bytes=100 * 1024 * 1024),
  )(A_x.reshape(1, D), gate_w.reshape(D // 128, 128), kt, vt, A_wq, A_wo, B_w1, B_w3, B_w2)
  return out.reshape(1, 1, D)
```

```python
import functools

import jax
import jax.numpy as jnp
from jax import lax
import jax.experimental.pallas as pl
import jax.experimental.pallas.tpu as pltpu

D = 640
HQ = 32
DH = 192
HD = HQ * DH
F = 1536
G = 2
GR = G * DH
NG = HQ // G
GA = 2
NB = 2 * GA
LROWS = 8
W2_SPLITS = (1024, 384, 128)
KV_CUT = (192, 128, (0, 1), "c")
NPART = 2
WQ_CUT = (128, 128, (0, 1), "r")
WO_CUT = (192, 640, (0, 1), "r")
W13_CUT = (128, 128, (0, 1), "r")
W2_CUT = (128, 128, (0, 1), "r")

COMPUTE = True
PRIME_ONLY = False
WAITX = "none"
SPIN = (0, 0, 0, 0)
INTERLEAVE = True
_NT = (((1,), (1,)), ((), ()))


def _start_cut(src, dst, sem, cut):
  sr, sc, pat, order = cut
  rows, cols = dst.shape
  sr, sc = min(sr, rows), min(sc, cols)
  assert rows % sr == 0 and cols % sc == 0, (dst.shape, cut)
  nr, nc = rows // sr, cols // sc
  n_out, n_in = (nr, nc) if order == "r" else (nc, nr)
  unroll = 1
  while (unroll * n_in) % len(pat):
    unroll += 1
  if n_out % unroll:
    unroll = n_out

  def burst(o):
    for u in range(unroll):
      for i in range(n_in):
        oo = o * unroll + u
        if order == "r":
          r, c = oo * sr, i * sc
          if not isinstance(r, int):
            r = pl.multiple_of(r, sr)
        else:
          r, c = i * sr, oo * sc
          if not isinstance(c, int):
            c = pl.multiple_of(c, sc)
        pltpu.make_async_copy(src.at[pl.ds(r, sr), pl.ds(c, sc)], dst.at[pl.ds(r, sr), pl.ds(c, sc)],
                              sem).start(priority=pat[(u * n_in + i) % len(pat)])

  if n_out // unroll == 1:
    burst(0)
  else:
    def body(o, carry):
      burst(o)
      return carry
    lax.fori_loop(0, n_out // unroll, body, 0)


def _wait_all(dst, sem):
  pltpu.make_async_copy(dst, dst, sem).wait()


def _kernel(x_hbm, gw_hbm, k_hbm, v_hbm, wq_hbm, wo_hbm, w1_hbm, w3_hbm, w2_hbm,
            o_ref,
            x_v, gw_v, wq_v, wo_v, w1_v, w3_v, w2_v, kv_v, q_s, base_s, s_s, p_s,
            sem_a, sem_kv, sem_wo, *, sk, win):
  col0 = sk - win
  scale = DH ** -0.5

  def rows_of(g):
    return pl.ds(g * GR, GR) if isinstance(g, int) else pl.ds(pl.multiple_of(g * GR, GR), GR)

  pw = win // NPART

  def kv_start(src, g, slot, part=None):
    if part is None:
      c0, n = 0, win
    elif isinstance(part, int):
      c0, n = part * pw, pw
    else:
      c0, n = pl.multiple_of(part * pw, pw), pw
    _start_cut(src.at[rows_of(g), pl.ds(col0 + c0, n)], kv_v.at[slot, :, pl.ds(c0, n)],
               sem_kv.at[slot], KV_CUT)

  def k_start(g, slot, part=None):
    kv_start(k_hbm, g, slot, part)

  def v_start(g, slot, part=None):
    kv_start(v_hbm, g, slot, part)

  def wo_start(g, slot):
    _start_cut(wo_hbm.at[rows_of(g), :], wo_v.at[rows_of(g), :], sem_wo.at[slot], WO_CUT)

  def wo_wait(g, slot):
    _wait_all(wo_v.at[rows_of(g), :], sem_wo.at[slot])

  cp_x = pltpu.make_async_copy(x_hbm, x_v, sem_a.at[0])
  cp_gw = pltpu.make_async_copy(gw_hbm, gw_v, sem_a.at[0])
  w2_offs = [sum(W2_SPLITS[:i]) for i in range(len(W2_SPLITS))]
  assert sum(W2_SPLITS) == F and len(W2_SPLITS) <= 3
  w2_sems = [sem_a.at[0], sem_a.at[1], sem_kv.at[2 * ((NG - GA) % GA)]]
  w2_dst = [w2_v.at[pl.ds(o, n), :] for o, n in zip(w2_offs, W2_SPLITS)]
  w2_src = [w2_hbm.at[pl.ds(o, n), :] for o, n in zip(w2_offs, W2_SPLITS)]

  _start_cut(wq_hbm, wq_v, sem_a.at[0], WQ_CUT)
  cp_x.start()
  cp_gw.start()
  for g in range(GA):
    k_start(g, 2 * g)
    wo_start(g, g)
    v_start(g, 2 * g + 1)
    if g == 0:
      _start_cut(w1_hbm, w1_v, sem_a.at[1], W13_CUT)
      _start_cut(w3_hbm, w3_v, sem_a.at[1], W13_CUT)

  def spin(n, c):
    if n:
      c = lax.fori_loop(0, n, lambda i, t: t * 1.0001 + 0.5, c)
      s_s[:, 0:128] = c
    return c

  if PRIME_ONLY:
    waits = {
        "wq": lambda: (_wait_all(wq_v, sem_a.at[0]), cp_x.wait(), cp_gw.wait()),
        "w13": lambda: (_wait_all(w1_v, sem_a.at[1]), _wait_all(w3_v, sem_a.at[1])),
        "k0": lambda: _wait_all(kv_v.at[0], sem_kv.at[0]),
        "v0": lambda: _wait_all(kv_v.at[1], sem_kv.at[1]),
        "k1": lambda: _wait_all(kv_v.at[2], sem_kv.at[2]),
        "v1": lambda: _wait_all(kv_v.at[3], sem_kv.at[3]),
        "wo0": lambda: wo_wait(0, 0),
        "wo1": lambda: wo_wait(1, 1),
    }
    if WAITX != "none":
      waits.pop(WAITX)()
    c0_ = spin(SPIN[0], jnp.zeros((8, 128), jnp.float32))
    for w in waits.values():
      w()
    o_ref[...] = x_v[...] + c0_[0:1, 0:1].astype(jnp.bfloat16)
    return

  if not COMPUTE:
    _wait_all(wq_v, sem_a.at[0]); cp_x.wait(); cp_gw.wait()
    _wait_all(w1_v, sem_a.at[1]); _wait_all(w3_v, sem_a.at[1])
    c_init = spin(SPIN[0], jnp.zeros((8, 128), jnp.float32))
    def group0(g, c):
      ks = 2 * lax.rem(g, GA); vs = ks + 1; ws = lax.rem(g, GA); more = g + GA < NG
      _wait_all(kv_v.at[ks], sem_kv.at[ks])
      c = spin(SPIN[1], c)
      @pl.when(more)
      def _():
        k_start(g + GA, ks)
      @pl.when(g + GA == NG)
      def _():
        for src, dst, sem in zip(w2_src, w2_dst, w2_sems):
          _start_cut(src, dst, sem, W2_CUT)
      wo_wait(g, ws)
      @pl.when(more)
      def _():
        wo_start(g + GA, ws)
      _wait_all(kv_v.at[vs], sem_kv.at[vs])
      c = spin(SPIN[2], c)
      @pl.when(more)
      def _():
        v_start(g + GA, vs)
      return c
    cc = lax.fori_loop(0, NG, group0, c_init)
    for i in range(len(W2_SPLITS)):
      _wait_all(w2_dst[i], w2_sems[i])
    cc = spin(SPIN[3], cc)
    o_ref[...] = x_v[...] + cc[0:1, 0:1].astype(jnp.bfloat16)
    return

  _wait_all(wq_v, sem_a.at[0])
  cp_x.wait()
  cp_gw.wait()
  x = x_v[...]
  x8 = jnp.broadcast_to(x, (LROWS, D))
  xf = x.astype(jnp.float32)
  gwf = gw_v[...].astype(jnp.float32)
  prod = xf[:, 0:128] * gwf[0:1, :]
  for r in range(1, D // 128):
    prod = prod + xf[:, r * 128:(r + 1) * 128] * gwf[r:r + 1, :]
  gate_logit = jnp.sum(prod, axis=-1, keepdims=True)
  gmix = jax.nn.sigmoid(gate_logit)

  row = lax.broadcasted_iota(jnp.int32, (LROWS, GR), 0)
  head_in_group = lax.broadcasted_iota(jnp.int32, (LROWS, GR), 1) // DH
  diag = row == head_in_group

  def q_proj(g, carry):
    qg = jnp.dot(x8, wq_v[:, rows_of(g)], preferred_element_type=jnp.float32)
    q_s[g] = jnp.where(diag, qg.astype(jnp.bfloat16).astype(jnp.float32), 0.0)
    return carry

  lax.fori_loop(0, NG, q_proj, 0)

  _wait_all(w1_v, sem_a.at[1])
  _wait_all(w3_v, sem_a.at[1])
  gate = jnp.dot(x8, w1_v[...], preferred_element_type=jnp.float32)
  up = jnp.dot(x8, w3_v[...], preferred_element_type=jnp.float32)
  gate = gate.astype(jnp.bfloat16).astype(jnp.float32)
  up = up.astype(jnp.bfloat16).astype(jnp.float32)
  h8 = (gate * jax.nn.sigmoid(gate) * up).astype(jnp.bfloat16)

  def cols(c):
    return pl.ds(pl.multiple_of(c * pw, pw), pw)

  def group(g, acc):
    ks = 2 * lax.rem(g, GA)
    vs = ks + 1
    ws = lax.rem(g, GA)
    more = g + GA < NG
    qb = q_s[g].astype(jnp.bfloat16)
    _wait_all(kv_v.at[ks], sem_kv.at[ks])

    def qk_part(c, carry):
      s_s[:, cols(c)] = jnp.dot(qb, kv_v[ks, :, cols(c)], preferred_element_type=jnp.float32)
      if INTERLEAVE:
        @pl.when(more)
        def _():
          k_start(g + GA, ks, c)
      return carry

    lax.fori_loop(0, NPART, qk_part, 0)
    if not INTERLEAVE:
      @pl.when(more)
      def _():
        lax.fori_loop(0, NPART, lambda c, _: k_start(g + GA, ks, c), None)

    @pl.when(g + GA == NG)
    def _():
      for src, dst, sem in zip(w2_src, w2_dst, w2_sems):
        _start_cut(src, dst, sem, W2_CUT)

    wo_wait(g, ws)

    @pl.when(more)
    def _():
      wo_start(g + GA, ws)

    s = s_s[...] * scale
    m = jnp.max(s, axis=-1, keepdims=True)
    e = jnp.exp(s - m)
    l = jnp.sum(e, axis=-1, keepdims=True)
    p_s[...] = e

    _wait_all(kv_v.at[vs], sem_kv.at[vs])

    def pv_part(c, r):
      r = r + lax.dot_general(p_s[:, cols(c)].astype(jnp.bfloat16), kv_v[vs, :, cols(c)], _NT,
                              preferred_element_type=jnp.float32)
      if INTERLEAVE:
        @pl.when(more)
        def _():
          v_start(g + GA, vs, c)
      return r

    r = lax.fori_loop(0, NPART, pv_part, jnp.zeros((LROWS, GR), jnp.float32))
    if not INTERLEAVE:
      @pl.when(more)
      def _():
        lax.fori_loop(0, NPART, lambda c, _: v_start(g + GA, vs, c), None)

    o = jnp.where(diag, r / l, 0.0).astype(jnp.bfloat16)
    return acc + jnp.dot(o, wo_v[rows_of(g), :], preferred_element_type=jnp.float32)

  acc = lax.fori_loop(0, NG, group, jnp.zeros((LROWS, D), jnp.float32))

  out = gmix * jnp.sum(acc, axis=0, keepdims=True)
  for i, (o_, n) in enumerate(zip(w2_offs, W2_SPLITS)):
    if i > 0:
      out = base_s[...]
    _wait_all(w2_dst[i], w2_sems[i])
    part = jnp.dot(h8[:, o_:o_ + n], w2_v[pl.ds(o_, n), :], preferred_element_type=jnp.float32)
    out = out + (1.0 - gmix) * part[0:1, :]
    if i + 1 < len(W2_SPLITS):
      base_s[...] = out
  o_ref[...] = out.astype(o_ref.dtype)


@jax.jit
def pallas_gated_mix__sliding_block_cached__glu_gated_swiglu__decode_kernel(
    A_x, A_k_cache, A_v_cache, A_wq, A_wo, B_x, B_w1, B_w3, B_w2, gate_w):
  del B_x
  sk = A_k_cache.shape[2]
  win = min(4096, max(256, sk // 4))
  assert A_k_cache.shape == (1, HQ, sk, DH) and A_x.shape == (1, 1, D)
  kt = jnp.swapaxes(A_k_cache, 2, 3).reshape(HD, sk)
  vt = jnp.swapaxes(A_v_cache, 2, 3).reshape(HD, sk)
  any_spec = pl.BlockSpec(memory_space=pl.ANY)
  bf16 = jnp.bfloat16
  out = pl.pallas_call(
      functools.partial(_kernel, sk=sk, win=win),
      out_shape=jax.ShapeDtypeStruct((1, D), A_x.dtype),
      in_specs=[any_spec] * 9,
      out_specs=pl.BlockSpec(memory_space=pltpu.VMEM),
      scratch_shapes=[
          pltpu.VMEM((1, D), bf16),
          pltpu.VMEM((D // 128, 128), bf16),
          pltpu.VMEM((D, HD), bf16),
          pltpu.VMEM((HD, D), bf16),
          pltpu.VMEM((D, F), bf16),
          pltpu.VMEM((D, F), bf16),
          pltpu.VMEM((F, D), bf16),
          pltpu.VMEM((NB, GR, win), bf16),
          pltpu.VMEM((NG, LROWS, GR), jnp.float32),
          pltpu.VMEM((1, D), jnp.float32),
          pltpu.VMEM((LROWS, win), jnp.float32),
          pltpu.VMEM((LROWS, win), jnp.float32),
          pltpu.SemaphoreType.DMA((2,)),
          pltpu.SemaphoreType.DMA((NB,)),
          pltpu.SemaphoreType.DMA((GA,)),
      ],
      compiler_params=pltpu.CompilerParams(vmem_limit_bytes=100 * 1024 * 1024),
  )(A_x.reshape(1, D), gate_w.reshape(D // 128, 128), kt, vt, A_wq, A_wo, B_w1, B_w3, B_w2)
  return out.reshape(1, 1, D)
```

```python
import functools

import jax
import jax.numpy as jnp
from jax import lax
import jax.experimental.pallas as pl
import jax.experimental.pallas.tpu as pltpu

D = 640
HQ = 32
DH = 192
HD = HQ * DH
F = 1536
G = 2
GR = G * DH
NG = HQ // G
GA = 2
NB = 2 * GA
LROWS = 8
W2_SPLITS = (1024, 384, 128)
W2_EARLY = False
WOD = 4
KV_SR = 192
KV_PAT = (0, 1)
WQ_CUT = (128, 128, (0, 1), "r")
WO_CUT = (192, 640, (0, 1), "r")
WO_LAST_CUT = (192, 640, (0, 1), "r")
W13_CUT = (128, 128, (0, 1), "r")
W2_CUT = (128, 128, (0, 1), "r")
COMPUTE = True
NOBC = False
SCOPES = False

_NT = (((1,), (1,)), ((), ()))


def _scope(name):
  import contextlib
  return jax.named_scope(name) if SCOPES else contextlib.nullcontext()


def _start_cut(src, dst, sem, cut):
  sr, sc, pat, order = cut
  rows, cols = dst.shape
  sr, sc = min(sr, rows), min(sc, cols)
  assert rows % sr == 0 and cols % sc == 0, (dst.shape, cut)
  nr, nc = rows // sr, cols // sc
  n_out, n_in = (nr, nc) if order == "r" else (nc, nr)
  unroll = 1
  while (unroll * n_in) % len(pat):
    unroll += 1
  if n_out % unroll:
    unroll = n_out

  def burst(o):
    for u in range(unroll):
      for i in range(n_in):
        oo = o * unroll + u
        if order == "r":
          r, c = oo * sr, i * sc
          if not isinstance(r, int):
            r = pl.multiple_of(r, sr)
        else:
          r, c = i * sr, oo * sc
          if not isinstance(c, int):
            c = pl.multiple_of(c, sc)
        pltpu.make_async_copy(src.at[pl.ds(r, sr), pl.ds(c, sc)], dst.at[pl.ds(r, sr), pl.ds(c, sc)],
                              sem).start(priority=pat[(u * n_in + i) % len(pat)])

  if n_out // unroll == 1:
    burst(0)
  else:
    def body(o, carry):
      burst(o)
      return carry
    lax.fori_loop(0, n_out // unroll, body, 0)


def _wait_all(dst, sem):
  pltpu.make_async_copy(dst, dst, sem).wait()


def _kernel(x_hbm, gw_hbm, k_hbm, v_hbm, wq_hbm, wo_hbm, w1_hbm, w3_hbm, w2_hbm,
            o_ref,
            x_v, gw_v, wq_v, wo_v, w1_v, w3_v, w2_v, kv_v, q_s, r_s, base_s,
            sem_a, sem_kv, sem_wo, *, sk, win):
  col0 = sk - win
  scale = DH ** -0.5
  ncb = win // 128

  def rows_of(g):
    return pl.ds(g * GR, GR) if isinstance(g, int) else pl.ds(pl.multiple_of(g * GR, GR), GR)

  def kv_start(src, g, slot):
    r0 = g * GR if isinstance(g, int) else pl.multiple_of(g * GR, GR)
    nr = GR // KV_SR
    unroll = 1
    while (unroll * nr) % len(KV_PAT):
      unroll += 1

    def body(t, carry):
      for u in range(unroll):
        cb = t * unroll + u
        for i in range(nr):
          pltpu.make_async_copy(
              src.at[pl.ds(r0 + i * KV_SR, KV_SR), pl.ds(pl.multiple_of(col0 + cb * 128, 128), 128)],
              kv_v.at[slot, cb, pl.ds(i * KV_SR, KV_SR), :],
              sem_kv.at[slot]).start(priority=KV_PAT[(u * nr + i) % len(KV_PAT)])
      return carry
    lax.fori_loop(0, ncb // unroll, body, 0)

  def kv_wait(slot):
    _wait_all(kv_v.at[slot], sem_kv.at[slot])

  def wo_start(g, slot, cut=None):
    _start_cut(wo_hbm.at[rows_of(g), :], wo_v.at[rows_of(g), :], sem_wo.at[slot], cut or WO_CUT)

  def wo_wait(g, slot):
    _wait_all(wo_v.at[rows_of(g), :], sem_wo.at[slot])

  cp_x = pltpu.make_async_copy(x_hbm, x_v, sem_a.at[0])
  cp_gw = pltpu.make_async_copy(gw_hbm, gw_v, sem_a.at[0])
  w2_offs = [sum(W2_SPLITS[:i]) for i in range(len(W2_SPLITS))]
  assert sum(W2_SPLITS) == F and len(W2_SPLITS) <= 3
  w2_sems = [sem_a.at[0], sem_a.at[1], sem_kv.at[2 * ((NG - GA) % GA)]]
  w2_dst = [w2_v.at[pl.ds(o, n), :] for o, n in zip(w2_offs, W2_SPLITS)]
  w2_src = [w2_hbm.at[pl.ds(o, n), :] for o, n in zip(w2_offs, W2_SPLITS)]

  with _scope("prime"):
    _start_cut(wq_hbm, wq_v, sem_a.at[0], WQ_CUT)
    cp_x.start()
    cp_gw.start()
    for g in range(GA):
      kv_start(k_hbm, g, 2 * g)
      kv_start(v_hbm, g, 2 * g + 1)
      if g == 0:
        _start_cut(w1_hbm, w1_v, sem_a.at[1], W13_CUT)
        _start_cut(w3_hbm, w3_v, sem_a.at[1], W13_CUT)
        if W2_EARLY:
          _start_cut(w2_hbm, w2_v, sem_a.at[1], W2_CUT)

  with _scope("qproj"):
    _wait_all(wq_v, sem_a.at[0])
    cp_x.wait()
    cp_gw.wait()
    x = x_v[...]
    x8 = jnp.broadcast_to(x, (LROWS, D))
    xf = x.astype(jnp.float32)
    gwf = gw_v[...].astype(jnp.float32)
    prod = xf[:, 0:128] * gwf[0:1, :]
    for r in range(1, D // 128):
      prod = prod + xf[:, r * 128:(r + 1) * 128] * gwf[r:r + 1, :]
    gate_logit = jnp.sum(prod, axis=-1, keepdims=True)
    gmix = jax.nn.sigmoid(gate_logit)

    row = lax.broadcasted_iota(jnp.int32, (LROWS, GR), 0)
    head_in_group = lax.broadcasted_iota(jnp.int32, (LROWS, GR), 1) // DH
    diag = row == head_in_group

    def q_proj(g, carry):
      qg = jnp.dot(x8, wq_v[:, rows_of(g)], preferred_element_type=jnp.float32)
      q_s[g] = jnp.where(diag, qg.astype(jnp.bfloat16).astype(jnp.float32), 0.0)
      return carry

    if COMPUTE:
      lax.fori_loop(0, NG, q_proj, 0)

  with _scope("ffn"):
    _wait_all(w1_v, sem_a.at[1])
    _wait_all(w3_v, sem_a.at[1])
    if W2_EARLY:
      _wait_all(w2_v, sem_a.at[1])
    gate = jnp.dot(x8, w1_v[...], preferred_element_type=jnp.float32)
    up = jnp.dot(x8, w3_v[...], preferred_element_type=jnp.float32)
    gate = gate.astype(jnp.bfloat16).astype(jnp.float32)
    up = up.astype(jnp.bfloat16).astype(jnp.float32)
    h8 = (gate * jax.nn.sigmoid(gate) * up).astype(jnp.bfloat16)
    if W2_EARLY:
      b = jnp.dot(h8, w2_v[...], preferred_element_type=jnp.float32)
      base_s[...] = (1.0 - gmix) * b[0:1, :]

  def group(g, carry):
    ks = 2 * lax.rem(g, GA)
    vs = ks + 1
    more = g + GA < NG
    qb = q_s[g].astype(jnp.bfloat16)
    with _scope("a_kwait"):
      kv_wait(ks)
    with _scope("b_qk"):
      if COMPUTE:
        s = jnp.concatenate([jnp.dot(qb, kv_v[ks, j], preferred_element_type=jnp.float32)
                             for j in range(ncb)], axis=1) * scale

    with _scope("c_kstart"):
      @pl.when(more)
      def _():
        kv_start(k_hbm, g + GA, ks)

      if not W2_EARLY:
        @pl.when(g + GA == NG)
        def _():
          for src, dst, sem in zip(w2_src, w2_dst, w2_sems):
            _start_cut(src, dst, sem, W2_CUT)

    with _scope("d_softmax"):
      if COMPUTE:
        m = jnp.max(s, axis=-1, keepdims=True)
        e = jnp.exp(s - m)
        l = jnp.sum(e, axis=-1, keepdims=True)
        p = e.astype(jnp.bfloat16)

    with _scope("f_vwait"):
      kv_wait(vs)
    with _scope("g_pv"):
      if COMPUTE:
        r = None
        for j in range(ncb):
          rj = lax.dot_general(p[:, j * 128:(j + 1) * 128], kv_v[vs, j], _NT,
                               preferred_element_type=jnp.float32)
          r = rj if r is None else r + rj
        r_s[g] = jnp.where(diag, r / l, 0.0)

    with _scope("h_vstart"):
      @pl.when(more)
      def _():
        kv_start(v_hbm, g + GA, vs)

      @pl.when(g + GA == NG)
      def _():
        for c in range(WOD):
          wo_start(c, c)
    return carry

  lax.fori_loop(0, NG, group, 0)

  with _scope("w2"):
    if not W2_EARLY:
      out = jnp.zeros((1, D), jnp.float32)
      for i, (o_, n) in enumerate(zip(w2_offs, W2_SPLITS)):
        if i > 0:
          out = base_s[...]
        _wait_all(w2_dst[i], w2_sems[i])
        part = jnp.dot(h8[:, o_:o_ + n], w2_v[pl.ds(o_, n), :], preferred_element_type=jnp.float32)
        base_s[...] = out + (1.0 - gmix) * part[0:1, :]

  def out_chunk(c, acc):
    slot = lax.rem(c, WOD)
    with _scope("wo_wait"):
      wo_wait(c, slot)
    with _scope("wo_mm"):
      acc = acc + jnp.dot(r_s[c].astype(jnp.bfloat16), wo_v[rows_of(c), :], preferred_element_type=jnp.float32)

    @pl.when(c + WOD < NG - 1)
    def _():
      wo_start(c + WOD, slot)

    @pl.when(c + WOD == NG - 1)
    def _():
      wo_start(NG - 1, slot, WO_LAST_CUT)
    return acc

  acc = lax.fori_loop(0, NG - 1, out_chunk, jnp.zeros((LROWS, D), jnp.float32))
  with _scope("last"):
    base_s[...] = base_s[...] + gmix * jnp.sum(acc, axis=0, keepdims=True)
    c = NG - 1
    wo_wait(c, c % WOD)
    a = jnp.dot(r_s[c].astype(jnp.bfloat16), wo_v[rows_of(c), :], preferred_element_type=jnp.float32)
    o_ref[...] = (base_s[...] + gmix * jnp.sum(a, axis=0, keepdims=True)).astype(o_ref.dtype)


@jax.jit
def pallas_gated_mix__sliding_block_cached__glu_gated_swiglu__decode_kernel(
    A_x, A_k_cache, A_v_cache, A_wq, A_wo, B_x, B_w1, B_w3, B_w2, gate_w):
  del B_x
  sk = A_k_cache.shape[2]
  win = min(4096, max(256, sk // 4))
  assert A_k_cache.shape == (1, HQ, sk, DH) and A_x.shape == (1, 1, D)
  kt = jnp.swapaxes(A_k_cache, 2, 3).reshape(HD, sk)
  vt = jnp.swapaxes(A_v_cache, 2, 3).reshape(HD, sk)
  any_spec = pl.BlockSpec(memory_space=pl.ANY)
  bf16 = jnp.bfloat16
  out = pl.pallas_call(
      functools.partial(_kernel, sk=sk, win=win),
      out_shape=jax.ShapeDtypeStruct((1, D), A_x.dtype),
      in_specs=[any_spec] * 9,
      out_specs=pl.BlockSpec(memory_space=pltpu.VMEM),
      scratch_shapes=[
          pltpu.VMEM((1, D), bf16),
          pltpu.VMEM((D // 128, 128), bf16),
          pltpu.VMEM((D, HD), bf16),
          pltpu.VMEM((HD, D), bf16),
          pltpu.VMEM((D, F), bf16),
          pltpu.VMEM((D, F), bf16),
          pltpu.VMEM((F, D), bf16),
          pltpu.VMEM((NB, win // 128, GR, 128), bf16),
          pltpu.VMEM((NG, LROWS, GR), jnp.float32),
          pltpu.VMEM((NG, LROWS, GR), jnp.float32),
          pltpu.VMEM((1, D), jnp.float32),
          pltpu.SemaphoreType.DMA((2,)),
          pltpu.SemaphoreType.DMA((NB,)),
          pltpu.SemaphoreType.DMA((WOD,)),
      ],
      compiler_params=pltpu.CompilerParams(vmem_limit_bytes=100 * 1024 * 1024, disable_bounds_checks=NOBC),
  )(A_x.reshape(1, D), gate_w.reshape(D // 128, 128), kt, vt, A_wq, A_wo, B_w1, B_w3, B_w2)
  return out.reshape(1, 1, D)
```

```python
import functools

import jax
import jax.numpy as jnp
from jax import lax
import jax.experimental.pallas as pl
import jax.experimental.pallas.tpu as pltpu

D = 640
HQ = 32
DH = 192
HD = HQ * DH
F = 1536
G = 2
GR = G * DH
NG = HQ // G
GA = 2
NB = 2 * GA
LROWS = 8
W2_SPLITS = (1024, 384, 128)
W2_EARLY = False
WOT = 3
WO_SLOT = 'k'
KV_SR = 192
KV_PAT = (0, 1)
WQ_CUT = (128, 128, (0, 1), "r")
WO_CUT = (32, 640, (0, 1), "rh")
WO_TAIL_CUT = (192, 640, (0, 1), "r")
WO_LAST_CUT = (192, 640, (0, 1), "r")
W13_CUT = (128, 128, (0, 1), "r")
W2_CUT = (128, 128, (0, 1), "r")
COMPUTE = True
NOBC = False
SCOPES = False

_NT = (((1,), (1,)), ((), ()))


def _scope(name):
  import contextlib
  return jax.named_scope(name) if SCOPES else contextlib.nullcontext()


def _start_cut(src, dst, sem, cut):
  sr, sc, pat, order = cut
  rows, cols = dst.shape
  sr, sc = min(sr, rows), min(sc, cols)
  assert rows % sr == 0 and cols % sc == 0, (dst.shape, cut)
  nr, nc = rows // sr, cols // sc
  n_out, n_in = (nr, nc) if order[0] == "r" else (nc, nr)
  halves = order.endswith("h") and n_out % 2 == 0
  if halves:
    n_out //= 2
  per = n_in * (2 if halves else 1)
  unroll = 1
  while (unroll * per) % len(pat):
    unroll += 1
  if n_out % unroll:
    unroll = n_out

  def burst(o):
    j = 0
    for u in range(unroll):
      for i in range(n_in):
        for h in range(2 if halves else 1):
          oo = o * unroll + u + h * n_out
          if order[0] == "r":
            r, c = oo * sr, i * sc
            if not isinstance(r, int):
              r = pl.multiple_of(r, sr)
          else:
            r, c = i * sr, oo * sc
            if not isinstance(c, int):
              c = pl.multiple_of(c, sc)
          pltpu.make_async_copy(src.at[pl.ds(r, sr), pl.ds(c, sc)], dst.at[pl.ds(r, sr), pl.ds(c, sc)],
                                sem).start(priority=pat[j % len(pat)])
          j += 1

  if n_out // unroll == 1:
    burst(0)
  else:
    def body(o, carry):
      burst(o)
      return carry
    lax.fori_loop(0, n_out // unroll, body, 0)


def _wait_all(dst, sem):
  pltpu.make_async_copy(dst, dst, sem).wait()


def _kernel(x_hbm, gw_hbm, k_hbm, v_hbm, wq_hbm, wo_hbm, w1_hbm, w3_hbm, w2_hbm,
            o_ref,
            x_v, gw_v, wq_v, wo_v, w1_v, w3_v, w2_v, kv_v, q_s, r_s, acc_s, base_s,
            sem_a, sem_kv, sem_wo, sem_wt, *, sk, win):
  col0 = sk - win
  scale = DH ** -0.5
  ncb = win // 128

  def rows_of(g):
    return pl.ds(g * GR, GR) if isinstance(g, int) else pl.ds(pl.multiple_of(g * GR, GR), GR)

  def kv_start(src, g, slot):
    r0 = g * GR if isinstance(g, int) else pl.multiple_of(g * GR, GR)
    nr = GR // KV_SR
    unroll = 1
    while (unroll * nr) % len(KV_PAT):
      unroll += 1

    def body(t, carry):
      for u in range(unroll):
        cb = t * unroll + u
        for i in range(nr):
          pltpu.make_async_copy(
              src.at[pl.ds(r0 + i * KV_SR, KV_SR), pl.ds(pl.multiple_of(col0 + cb * 128, 128), 128)],
              kv_v.at[slot, cb, pl.ds(i * KV_SR, KV_SR), :],
              sem_kv.at[slot]).start(priority=KV_PAT[(u * nr + i) % len(KV_PAT)])
      return carry
    lax.fori_loop(0, ncb // unroll, body, 0)

  def kv_wait(slot):
    _wait_all(kv_v.at[slot], sem_kv.at[slot])

  def wo_start(g, sem, cut):
    _start_cut(wo_hbm.at[rows_of(g), :], wo_v.at[rows_of(g), :], sem, cut)

  def wo_wait(g, sem):
    _wait_all(wo_v.at[rows_of(g), :], sem)

  NI = NG - WOT

  cp_x = pltpu.make_async_copy(x_hbm, x_v, sem_a.at[0])
  cp_gw = pltpu.make_async_copy(gw_hbm, gw_v, sem_a.at[0])
  w2_offs = [sum(W2_SPLITS[:i]) for i in range(len(W2_SPLITS))]
  assert sum(W2_SPLITS) == F and len(W2_SPLITS) <= 3
  w2_sems = [sem_a.at[0], sem_a.at[1], sem_kv.at[2 * ((NG - GA) % GA)]]
  w2_dst = [w2_v.at[pl.ds(o, n), :] for o, n in zip(w2_offs, W2_SPLITS)]
  w2_src = [w2_hbm.at[pl.ds(o, n), :] for o, n in zip(w2_offs, W2_SPLITS)]

  with _scope("prime"):
    _start_cut(wq_hbm, wq_v, sem_a.at[0], WQ_CUT)
    cp_x.start()
    cp_gw.start()
    for g in range(GA):
      kv_start(k_hbm, g, 2 * g)
      if g < NI and WO_SLOT == 'k':
        wo_start(g, sem_wo.at[g], WO_CUT)
      kv_start(v_hbm, g, 2 * g + 1)
      if g < NI and WO_SLOT == 'v':
        wo_start(g, sem_wo.at[g], WO_CUT)
      if g == 0:
        _start_cut(w1_hbm, w1_v, sem_a.at[1], W13_CUT)
        _start_cut(w3_hbm, w3_v, sem_a.at[1], W13_CUT)
        if W2_EARLY:
          _start_cut(w2_hbm, w2_v, sem_a.at[1], W2_CUT)

  with _scope("qproj"):
    _wait_all(wq_v, sem_a.at[0])
    cp_x.wait()
    cp_gw.wait()
    x = x_v[...]
    x8 = jnp.broadcast_to(x, (LROWS, D))
    xf = x.astype(jnp.float32)
    gwf = gw_v[...].astype(jnp.float32)
    prod = xf[:, 0:128] * gwf[0:1, :]
    for r in range(1, D // 128):
      prod = prod + xf[:, r * 128:(r + 1) * 128] * gwf[r:r + 1, :]
    gate_logit = jnp.sum(prod, axis=-1, keepdims=True)
    gmix = jax.nn.sigmoid(gate_logit)

    row = lax.broadcasted_iota(jnp.int32, (LROWS, GR), 0)
    head_in_group = lax.broadcasted_iota(jnp.int32, (LROWS, GR), 1) // DH
    diag = row == head_in_group

    def q_proj(g, carry):
      qg = jnp.dot(x8, wq_v[:, rows_of(g)], preferred_element_type=jnp.float32)
      q_s[g] = jnp.where(diag, qg.astype(jnp.bfloat16).astype(jnp.float32), 0.0)
      return carry

    if COMPUTE:
      lax.fori_loop(0, NG, q_proj, 0)

  with _scope("ffn"):
    _wait_all(w1_v, sem_a.at[1])
    _wait_all(w3_v, sem_a.at[1])
    if W2_EARLY:
      _wait_all(w2_v, sem_a.at[1])
    gate = jnp.dot(x8, w1_v[...], preferred_element_type=jnp.float32)
    up = jnp.dot(x8, w3_v[...], preferred_element_type=jnp.float32)
    gate = gate.astype(jnp.bfloat16).astype(jnp.float32)
    up = up.astype(jnp.bfloat16).astype(jnp.float32)
    h8 = (gate * jax.nn.sigmoid(gate) * up).astype(jnp.bfloat16)
    if W2_EARLY:
      b = jnp.dot(h8, w2_v[...], preferred_element_type=jnp.float32)
      base_s[...] = (1.0 - gmix) * b[0:1, :]

  def wo_turn(g):
    ws = lax.rem(g, GA)

    @pl.when(g < NI)
    def _():
      wo_wait(g, sem_wo.at[ws])

    @pl.when(g + GA < NI)
    def _():
      wo_start(g + GA, sem_wo.at[ws], WO_CUT)

  acc_s[...] = jnp.zeros_like(acc_s)

  def group(g, carry):
    ks = 2 * lax.rem(g, GA)
    vs = ks + 1
    more = g + GA < NG
    qb = q_s[g].astype(jnp.bfloat16)
    with _scope("a_kwait"):
      kv_wait(ks)
    with _scope("b_qk"):
      if COMPUTE:
        s = jnp.concatenate([jnp.dot(qb, kv_v[ks, j], preferred_element_type=jnp.float32)
                             for j in range(ncb)], axis=1) * scale

    with _scope("c_kstart"):
      @pl.when(more)
      def _():
        kv_start(k_hbm, g + GA, ks)

      if WO_SLOT == 'k':
        wo_turn(g)

      if not W2_EARLY:
        @pl.when(g + GA == NG)
        def _():
          for src, dst, sem in zip(w2_src, w2_dst, w2_sems):
            _start_cut(src, dst, sem, W2_CUT)

    with _scope("d_softmax"):
      if COMPUTE:
        m = jnp.max(s, axis=-1, keepdims=True)
        e = jnp.exp(s - m)
        l = jnp.sum(e, axis=-1, keepdims=True)
        p = e.astype(jnp.bfloat16)

    with _scope("f_vwait"):
      kv_wait(vs)
    with _scope("g_pv"):
      if COMPUTE:
        r = None
        for j in range(ncb):
          rj = lax.dot_general(p[:, j * 128:(j + 1) * 128], kv_v[vs, j], _NT,
                               preferred_element_type=jnp.float32)
          r = rj if r is None else r + rj
        o = jnp.where(diag, r / l, 0.0)

    with _scope("h_vstart"):
      @pl.when(more)
      def _():
        kv_start(v_hbm, g + GA, vs)

      if WO_SLOT == 'v':
        wo_turn(g)

      @pl.when(g + GA == NG)
      def _():
        for c in range(WOT):
          wo_start(NI + c, sem_wt.at[c], WO_LAST_CUT if c == WOT - 1 else WO_TAIL_CUT)

    with _scope("i_oproj"):
      if COMPUTE:
        @pl.when(g < NI)
        def _():
          acc_s[...] += jnp.dot(o.astype(jnp.bfloat16), wo_v[rows_of(g), :], preferred_element_type=jnp.float32)

        @pl.when(g >= NI)
        def _():
          r_s[jnp.maximum(g - NI, 0)] = o
    return carry

  lax.fori_loop(0, NG, group, 0)

  with _scope("w2"):
    if not W2_EARLY:
      out = jnp.zeros((1, D), jnp.float32)
      for i, (o_, n) in enumerate(zip(w2_offs, W2_SPLITS)):
        if i > 0:
          out = base_s[...]
        _wait_all(w2_dst[i], w2_sems[i])
        part = jnp.dot(h8[:, o_:o_ + n], w2_v[pl.ds(o_, n), :], preferred_element_type=jnp.float32)
        base_s[...] = out + (1.0 - gmix) * part[0:1, :]

  base = base_s[...] + gmix * jnp.sum(acc_s[...], axis=0, keepdims=True)
  base_s[...] = base
  for c in range(WOT):
    with _scope("wo_wait"):
      wo_wait(NI + c, sem_wt.at[c])
    with _scope("wo_mm"):
      a = jnp.dot(r_s[c].astype(jnp.bfloat16), wo_v[rows_of(NI + c), :], preferred_element_type=jnp.float32)
      base = base_s[...] + gmix * jnp.sum(a, axis=0, keepdims=True)
      if c + 1 < WOT:
        base_s[...] = base
  o_ref[...] = base.astype(o_ref.dtype)


@jax.jit
def pallas_gated_mix__sliding_block_cached__glu_gated_swiglu__decode_kernel(
    A_x, A_k_cache, A_v_cache, A_wq, A_wo, B_x, B_w1, B_w3, B_w2, gate_w):
  del B_x
  sk = A_k_cache.shape[2]
  win = min(4096, max(256, sk // 4))
  assert A_k_cache.shape == (1, HQ, sk, DH) and A_x.shape == (1, 1, D)
  kt = jnp.swapaxes(A_k_cache, 2, 3).reshape(HD, sk)
  vt = jnp.swapaxes(A_v_cache, 2, 3).reshape(HD, sk)
  any_spec = pl.BlockSpec(memory_space=pl.ANY)
  bf16 = jnp.bfloat16
  out = pl.pallas_call(
      functools.partial(_kernel, sk=sk, win=win),
      out_shape=jax.ShapeDtypeStruct((1, D), A_x.dtype),
      in_specs=[any_spec] * 9,
      out_specs=pl.BlockSpec(memory_space=pltpu.VMEM),
      scratch_shapes=[
          pltpu.VMEM((1, D), bf16),
          pltpu.VMEM((D // 128, 128), bf16),
          pltpu.VMEM((D, HD), bf16),
          pltpu.VMEM((HD, D), bf16),
          pltpu.VMEM((D, F), bf16),
          pltpu.VMEM((D, F), bf16),
          pltpu.VMEM((F, D), bf16),
          pltpu.VMEM((NB, win // 128, GR, 128), bf16),
          pltpu.VMEM((NG, LROWS, GR), jnp.float32),
          pltpu.VMEM((WOT, LROWS, GR), jnp.float32),
          pltpu.VMEM((LROWS, D), jnp.float32),
          pltpu.VMEM((1, D), jnp.float32),
          pltpu.SemaphoreType.DMA((2,)),
          pltpu.SemaphoreType.DMA((NB,)),
          pltpu.SemaphoreType.DMA((GA,)),
          pltpu.SemaphoreType.DMA((WOT,)),
      ],
      compiler_params=pltpu.CompilerParams(vmem_limit_bytes=100 * 1024 * 1024, disable_bounds_checks=NOBC),
  )(A_x.reshape(1, D), gate_w.reshape(D // 128, 128), kt, vt, A_wq, A_wo, B_w1, B_w3, B_w2)
  return out.reshape(1, 1, D)
```

```python
import functools

import jax
import jax.numpy as jnp
from jax import lax
import jax.experimental.pallas as pl
import jax.experimental.pallas.tpu as pltpu

D = 640
HQ = 32
DH = 192
HD = HQ * DH
F = 1536
G = 2
GR = G * DH
NG = HQ // G
GA = 2
NB = 2 * GA
LROWS = 8
W2_SPLITS = (1536,)
W2_EARLY = False
WOT = 3
WO_SLOT = 'k'
KV_SR = 192
KV_PAT = (0, 1)
LAST_K = None
LAST_V = None
WQ_CUT = (8, 1024, (0, 1), "rh")
WO_CUT = (48, 640, (0, 1), "rh")
WO_TAIL_CUT = (32, 640, (0, 1), "rh")
WO_LAST_CUT = (48, 640, (0, 1), "rh")
W13_CUT = (8, 768, (0, 1), "rh")
W2_CUT = (16, 640, (0, 1), "rh")
COMPUTE = True
NOBC = False
SCOPES = False

_NT = (((1,), (1,)), ((), ()))


def _scope(name):
  import contextlib
  return jax.named_scope(name) if SCOPES else contextlib.nullcontext()


def _start_cut(src, dst, sem, cut):
  sr, sc, pat, order = cut
  rows, cols = dst.shape
  sr, sc = min(sr, rows), min(sc, cols)
  assert rows % sr == 0 and cols % sc == 0, (dst.shape, cut)
  nr, nc = rows // sr, cols // sc
  n_out, n_in = (nr, nc) if order[0] == "r" else (nc, nr)
  halves = order.endswith("h") and n_out % 2 == 0
  if halves:
    n_out //= 2
  per = n_in * (2 if halves else 1)
  unroll = 1
  while (unroll * per) % len(pat):
    unroll += 1
  if n_out % unroll:
    unroll = n_out

  def burst(o):
    j = 0
    for u in range(unroll):
      for i in range(n_in):
        for h in range(2 if halves else 1):
          oo = o * unroll + u + h * n_out
          if order[0] == "r":
            r, c = oo * sr, i * sc
            if not isinstance(r, int):
              r = pl.multiple_of(r, sr)
          else:
            r, c = i * sr, oo * sc
            if not isinstance(c, int):
              c = pl.multiple_of(c, sc)
          pltpu.make_async_copy(src.at[pl.ds(r, sr), pl.ds(c, sc)], dst.at[pl.ds(r, sr), pl.ds(c, sc)],
                                sem).start(priority=pat[j % len(pat)])
          j += 1

  if n_out // unroll == 1:
    burst(0)
  else:
    def body(o, carry):
      burst(o)
      return carry
    lax.fori_loop(0, n_out // unroll, body, 0)


def _wait_all(dst, sem):
  pltpu.make_async_copy(dst, dst, sem).wait()


def _kernel(x_hbm, gw_hbm, k_hbm, v_hbm, wq_hbm, wo_hbm, w1_hbm, w3_hbm, w2_hbm,
            o_ref,
            x_v, gw_v, wq_v, wo_v, w1_v, w3_v, w2_v, kv_v, q_s, r_s, acc_s, base_s,
            sem_a, sem_kv, sem_wo, sem_wt, *, sk, win):
  col0 = sk - win
  SR0, PAT0 = KV_SR, KV_PAT
  scale = DH ** -0.5
  ncb = win // 128

  def rows_of(g):
    return pl.ds(g * GR, GR) if isinstance(g, int) else pl.ds(pl.multiple_of(g * GR, GR), GR)

  def kv_start(src, g, slot, mode=None):
    r0 = g * GR if isinstance(g, int) else pl.multiple_of(g * GR, GR)
    KV_SR, KV_PAT = mode or (SR0, PAT0)
    nr = GR // KV_SR
    unroll = 1
    while (unroll * nr) % len(KV_PAT):
      unroll += 1
    assert ncb % unroll == 0

    def body(t, carry):
      for u in range(unroll):
        cb = t * unroll + u
        for i in range(nr):
          pltpu.make_async_copy(
              src.at[pl.ds(r0 + i * KV_SR, KV_SR), pl.ds(pl.multiple_of(col0 + cb * 128, 128), 128)],
              kv_v.at[slot, cb, pl.ds(i * KV_SR, KV_SR), :],
              sem_kv.at[slot]).start(priority=KV_PAT[(u * nr + i) % len(KV_PAT)])
      return carry
    lax.fori_loop(0, ncb // unroll, body, 0)

  def kv_wait(slot):
    _wait_all(kv_v.at[slot], sem_kv.at[slot])

  def wo_start(g, sem, cut):
    _start_cut(wo_hbm.at[rows_of(g), :], wo_v.at[rows_of(g), :], sem, cut)

  def wo_wait(g, sem):
    _wait_all(wo_v.at[rows_of(g), :], sem)

  NI = NG - WOT

  cp_x = pltpu.make_async_copy(x_hbm, x_v, sem_a.at[0])
  cp_gw = pltpu.make_async_copy(gw_hbm, gw_v, sem_a.at[0])
  w2_offs = [sum(W2_SPLITS[:i]) for i in range(len(W2_SPLITS))]
  assert sum(W2_SPLITS) == F and len(W2_SPLITS) <= 3
  w2_sems = [sem_a.at[0], sem_a.at[1], sem_kv.at[2 * ((NG - GA) % GA)]]
  w2_dst = [w2_v.at[pl.ds(o, n), :] for o, n in zip(w2_offs, W2_SPLITS)]
  w2_src = [w2_hbm.at[pl.ds(o, n), :] for o, n in zip(w2_offs, W2_SPLITS)]

  with _scope("prime"):
    _start_cut(wq_hbm, wq_v, sem_a.at[0], WQ_CUT)
    cp_x.start()
    cp_gw.start()
    for g in range(GA):
      kv_start(k_hbm, g, 2 * g)
      if g < NI and WO_SLOT == 'k':
        wo_start(g, sem_wo.at[g], WO_CUT)
      kv_start(v_hbm, g, 2 * g + 1)
      if g < NI and WO_SLOT == 'v':
        wo_start(g, sem_wo.at[g], WO_CUT)
      if g == 0:
        _start_cut(w1_hbm, w1_v, sem_a.at[1], W13_CUT)
        _start_cut(w3_hbm, w3_v, sem_a.at[1], W13_CUT)
        if W2_EARLY:
          _start_cut(w2_hbm, w2_v, sem_a.at[1], W2_CUT)

  with _scope("qproj"):
    _wait_all(wq_v, sem_a.at[0])
    cp_x.wait()
    cp_gw.wait()
    x = x_v[...]
    x8 = jnp.broadcast_to(x, (LROWS, D))
    xf = x.astype(jnp.float32)
    gwf = gw_v[...].astype(jnp.float32)
    prod = xf[:, 0:128] * gwf[0:1, :]
    for r in range(1, D // 128):
      prod = prod + xf[:, r * 128:(r + 1) * 128] * gwf[r:r + 1, :]
    gate_logit = jnp.sum(prod, axis=-1, keepdims=True)
    gmix = jax.nn.sigmoid(gate_logit)

    row = lax.broadcasted_iota(jnp.int32, (LROWS, GR), 0)
    head_in_group = lax.broadcasted_iota(jnp.int32, (LROWS, GR), 1) // DH
    diag = row == head_in_group

    def q_proj(g, carry):
      qg = jnp.dot(x8, wq_v[:, rows_of(g)], preferred_element_type=jnp.float32)
      q_s[g] = jnp.where(diag, qg.astype(jnp.bfloat16).astype(jnp.float32), 0.0)
      return carry

    if COMPUTE:
      lax.fori_loop(0, NG, q_proj, 0)

  with _scope("ffn"):
    _wait_all(w1_v, sem_a.at[1])
    _wait_all(w3_v, sem_a.at[1])
    if W2_EARLY:
      _wait_all(w2_v, sem_a.at[1])
    gate = jnp.dot(x8, w1_v[...], preferred_element_type=jnp.float32)
    up = jnp.dot(x8, w3_v[...], preferred_element_type=jnp.float32)
    gate = gate.astype(jnp.bfloat16).astype(jnp.float32)
    up = up.astype(jnp.bfloat16).astype(jnp.float32)
    h8 = (gate * jax.nn.sigmoid(gate) * up).astype(jnp.bfloat16)
    if W2_EARLY:
      b = jnp.dot(h8, w2_v[...], preferred_element_type=jnp.float32)
      base_s[...] = (1.0 - gmix) * b[0:1, :]

  def wo_turn(g):
    ws = lax.rem(g, GA)

    @pl.when(g < NI)
    def _():
      wo_wait(g, sem_wo.at[ws])

    @pl.when(g + GA < NI)
    def _():
      wo_start(g + GA, sem_wo.at[ws], WO_CUT)

  acc_s[...] = jnp.zeros_like(acc_s)

  def group(g, carry):
    ks = 2 * lax.rem(g, GA)
    vs = ks + 1
    more = g + GA < NG
    qb = q_s[g].astype(jnp.bfloat16)
    with _scope("a_kwait"):
      kv_wait(ks)
    with _scope("b_qk"):
      if COMPUTE:
        s = jnp.concatenate([jnp.dot(qb, kv_v[ks, j], preferred_element_type=jnp.float32)
                             for j in range(ncb)], axis=1) * scale

    with _scope("c_kstart"):
      @pl.when(more if LAST_K is None else g + GA < NG - 1)
      def _():
        kv_start(k_hbm, g + GA, ks)

      if LAST_K is not None:
        @pl.when(g + GA == NG - 1)
        def _():
          kv_start(k_hbm, NG - 1, ks, LAST_K)

      if WO_SLOT == 'k':
        wo_turn(g)

      if not W2_EARLY:
        @pl.when(g + GA == NG)
        def _():
          for src, dst, sem in zip(w2_src, w2_dst, w2_sems):
            _start_cut(src, dst, sem, W2_CUT)

    with _scope("d_softmax"):
      if COMPUTE:
        m = jnp.max(s, axis=-1, keepdims=True)
        e = jnp.exp(s - m)
        l = jnp.sum(e, axis=-1, keepdims=True)
        p = e.astype(jnp.bfloat16)

    with _scope("f_vwait"):
      kv_wait(vs)
    with _scope("g_pv"):
      if COMPUTE:
        r = None
        for j in range(ncb):
          rj = lax.dot_general(p[:, j * 128:(j + 1) * 128], kv_v[vs, j], _NT,
                               preferred_element_type=jnp.float32)
          r = rj if r is None else r + rj
        o = jnp.where(diag, r / l, 0.0)

    with _scope("h_vstart"):
      @pl.when(more if LAST_V is None else g + GA < NG - 1)
      def _():
        kv_start(v_hbm, g + GA, vs)

      if LAST_V is not None:
        @pl.when(g + GA == NG - 1)
        def _():
          kv_start(v_hbm, NG - 1, vs, LAST_V)

      if WO_SLOT == 'v':
        wo_turn(g)

      @pl.when(g + GA == NG)
      def _():
        for c in range(WOT):
          wo_start(NI + c, sem_wt.at[c], WO_LAST_CUT if c == WOT - 1 else WO_TAIL_CUT)

    with _scope("i_oproj"):
      if COMPUTE:
        @pl.when(g < NI)
        def _():
          acc_s[...] += jnp.dot(o.astype(jnp.bfloat16), wo_v[rows_of(g), :], preferred_element_type=jnp.float32)

        @pl.when(g >= NI)
        def _():
          r_s[jnp.maximum(g - NI, 0)] = o
    return carry

  lax.fori_loop(0, NG, group, 0)

  with _scope("w2"):
    if not W2_EARLY:
      out = jnp.zeros((1, D), jnp.float32)
      for i, (o_, n) in enumerate(zip(w2_offs, W2_SPLITS)):
        if i > 0:
          out = base_s[...]
        _wait_all(w2_dst[i], w2_sems[i])
        part = jnp.dot(h8[:, o_:o_ + n], w2_v[pl.ds(o_, n), :], preferred_element_type=jnp.float32)
        base_s[...] = out + (1.0 - gmix) * part[0:1, :]

  base = base_s[...] + gmix * jnp.sum(acc_s[...], axis=0, keepdims=True)
  base_s[...] = base
  for c in range(WOT):
    with _scope("wo_wait"):
      wo_wait(NI + c, sem_wt.at[c])
    with _scope("wo_mm"):
      a = jnp.dot(r_s[c].astype(jnp.bfloat16), wo_v[rows_of(NI + c), :], preferred_element_type=jnp.float32)
      base = base_s[...] + gmix * jnp.sum(a, axis=0, keepdims=True)
      if c + 1 < WOT:
        base_s[...] = base
  o_ref[...] = base.astype(o_ref.dtype)


@jax.jit
def pallas_gated_mix__sliding_block_cached__glu_gated_swiglu__decode_kernel(
    A_x, A_k_cache, A_v_cache, A_wq, A_wo, B_x, B_w1, B_w3, B_w2, gate_w):
  del B_x
  sk = A_k_cache.shape[2]
  win = min(4096, max(256, sk // 4))
  assert A_k_cache.shape == (1, HQ, sk, DH) and A_x.shape == (1, 1, D)
  kt = jnp.swapaxes(A_k_cache, 2, 3).reshape(HD, sk)
  vt = jnp.swapaxes(A_v_cache, 2, 3).reshape(HD, sk)
  any_spec = pl.BlockSpec(memory_space=pl.ANY)
  bf16 = jnp.bfloat16
  out = pl.pallas_call(
      functools.partial(_kernel, sk=sk, win=win),
      out_shape=jax.ShapeDtypeStruct((1, D), A_x.dtype),
      in_specs=[any_spec] * 9,
      out_specs=pl.BlockSpec(memory_space=pltpu.VMEM),
      scratch_shapes=[
          pltpu.VMEM((1, D), bf16),
          pltpu.VMEM((D // 128, 128), bf16),
          pltpu.VMEM((D, HD), bf16),
          pltpu.VMEM((HD, D), bf16),
          pltpu.VMEM((D, F), bf16),
          pltpu.VMEM((D, F), bf16),
          pltpu.VMEM((F, D), bf16),
          pltpu.VMEM((NB, win // 128, GR, 128), bf16),
          pltpu.VMEM((NG, LROWS, GR), jnp.float32),
          pltpu.VMEM((WOT, LROWS, GR), jnp.float32),
          pltpu.VMEM((LROWS, D), jnp.float32),
          pltpu.VMEM((1, D), jnp.float32),
          pltpu.SemaphoreType.DMA((2,)),
          pltpu.SemaphoreType.DMA((NB,)),
          pltpu.SemaphoreType.DMA((GA,)),
          pltpu.SemaphoreType.DMA((WOT,)),
      ],
      compiler_params=pltpu.CompilerParams(vmem_limit_bytes=100 * 1024 * 1024, disable_bounds_checks=NOBC),
  )(A_x.reshape(1, D), gate_w.reshape(D // 128, 128), kt, vt, A_wq, A_wo, B_w1, B_w3, B_w2)
  return out.reshape(1, 1, D)
```

```python
import functools

import jax
import jax.numpy as jnp
from jax import lax
import jax.experimental.pallas as pl
import jax.experimental.pallas.tpu as pltpu

D = 640
HQ = 32
DH = 192
HD = HQ * DH
F = 1536
G = 2
GR = G * DH
NG = HQ // G
GA = 2
LROWS = 8
NT = 3

KV_SUB = (192, 128)
WQ_SUB = (8, 1024)
W13_SUB = (8, 768)
W2_SUB = (16, 640)
WO_SUB = (48, 640)
WO_TAIL_SUB = (32, 640)
WO_LAST_SUB = (48, 640)

_NT_DIMS = (((1,), (1,)), ((), ()))


def _start_block(src, dst, sem, sub):
  rows, cols = dst.shape
  sr, sc = sub
  assert rows % (2 * sr) == 0 and cols % sc == 0, (dst.shape, sub)
  n = rows // (2 * sr)

  def burst(o):
    for ci in range(cols // sc):
      for h in range(2):
        r = o * sr + h * (rows // 2)
        if not isinstance(r, int):
          r = pl.multiple_of(r, sr)
        pltpu.make_async_copy(src.at[pl.ds(r, sr), pl.ds(ci * sc, sc)],
                              dst.at[pl.ds(r, sr), pl.ds(ci * sc, sc)], sem).start(priority=h)

  if n == 1:
    burst(0)
  else:
    def body(o, carry):
      burst(o)
      return carry
    lax.fori_loop(0, n, body, 0)


def _wait_block(dst, sem):
  pltpu.make_async_copy(dst, dst, sem).wait()


def _kernel(x_hbm, gw_hbm, k_hbm, v_hbm, wq_hbm, wo_hbm, w1_hbm, w3_hbm, w2_hbm,
            o_ref,
            x_v, gw_v, wq_v, wo_v, w1_v, w3_v, w2_v, kv_v, q_s, r_s, acc_s, out_s,
            sem_w, sem_kv, sem_wo, *, sk, win):
  col0 = sk - win
  ncb = win // 128
  scale = DH ** -0.5
  ni = NG - NT

  def rows_of(g):
    return pl.ds(g * GR, GR) if isinstance(g, int) else pl.ds(pl.multiple_of(g * GR, GR), GR)

  def kv_start(src, g, slot):
    sr = KV_SUB[0]
    r0 = g * GR if isinstance(g, int) else pl.multiple_of(g * GR, GR)

    def body(cb, carry):
      for i in range(GR // sr):
        pltpu.make_async_copy(
            src.at[pl.ds(r0 + i * sr, sr), pl.ds(pl.multiple_of(col0 + cb * 128, 128), 128)],
            kv_v.at[slot, cb, pl.ds(i * sr, sr), :],
            sem_kv.at[slot]).start(priority=i % 2)
      return carry
    lax.fori_loop(0, ncb, body, 0)

  def wo_start(rows, sem, sub):
    _start_block(wo_hbm.at[rows, :], wo_v.at[rows, :], sem, sub)

  tail_sems = [sem_wo.at[0], sem_wo.at[1], sem_w.at[1]]
  tail = [(g, WO_LAST_SUB if g == NG - 1 else WO_TAIL_SUB) for g in range(ni, NG)]
  assert len(tail) <= len(tail_sems) and NT >= GA

  cp_x = pltpu.make_async_copy(x_hbm, x_v, sem_w.at[0])
  cp_gw = pltpu.make_async_copy(gw_hbm, gw_v, sem_w.at[0])

  _start_block(wq_hbm, wq_v, sem_w.at[0], WQ_SUB)
  cp_x.start()
  cp_gw.start()
  for g in range(GA):
    kv_start(k_hbm, g, 2 * g)
    wo_start(rows_of(g), sem_wo.at[g], WO_SUB)
    kv_start(v_hbm, g, 2 * g + 1)
    if g == 0:
      _start_block(w1_hbm, w1_v, sem_w.at[1], W13_SUB)
      _start_block(w3_hbm, w3_v, sem_w.at[1], W13_SUB)

  _wait_block(wq_v, sem_w.at[0])
  cp_x.wait()
  cp_gw.wait()
  x = x_v[...]
  x8 = jnp.broadcast_to(x, (LROWS, D))
  xf = x.astype(jnp.float32)
  gwf = gw_v[...].astype(jnp.float32)
  prod = xf[:, 0:128] * gwf[0:1, :]
  for r in range(1, D // 128):
    prod = prod + xf[:, r * 128:(r + 1) * 128] * gwf[r:r + 1, :]
  gmix = jax.nn.sigmoid(jnp.sum(prod, axis=-1, keepdims=True))

  row = lax.broadcasted_iota(jnp.int32, (LROWS, GR), 0)
  head_in_group = lax.broadcasted_iota(jnp.int32, (LROWS, GR), 1) // DH
  diag = row == head_in_group

  def q_proj(g, carry):
    qg = jnp.dot(x8, wq_v[:, rows_of(g)], preferred_element_type=jnp.float32)
    q_s[g] = jnp.where(diag, qg.astype(jnp.bfloat16).astype(jnp.float32), 0.0)
    return carry

  lax.fori_loop(0, NG, q_proj, 0)

  _wait_block(w1_v, sem_w.at[1])
  _wait_block(w3_v, sem_w.at[1])
  gate = jnp.dot(x8, w1_v[...], preferred_element_type=jnp.float32)
  up = jnp.dot(x8, w3_v[...], preferred_element_type=jnp.float32)
  gate = gate.astype(jnp.bfloat16).astype(jnp.float32)
  up = up.astype(jnp.bfloat16).astype(jnp.float32)
  h8 = (gate * jax.nn.sigmoid(gate) * up).astype(jnp.bfloat16)

  acc_s[...] = jnp.zeros_like(acc_s)

  def group(g, carry):
    ks = 2 * lax.rem(g, GA)
    vs = ks + 1
    ws = lax.rem(g, GA)
    more = g + GA < NG
    qb = q_s[g].astype(jnp.bfloat16)
    _wait_block(kv_v.at[ks], sem_kv.at[ks])
    s = jnp.concatenate([jnp.dot(qb, kv_v[ks, j], preferred_element_type=jnp.float32)
                         for j in range(ncb)], axis=1) * scale

    @pl.when(more)
    def _():
      kv_start(k_hbm, g + GA, ks)

    @pl.when(g < ni)
    def _():
      _wait_block(wo_v.at[rows_of(g), :], sem_wo.at[ws])

    @pl.when(g + GA < ni)
    def _():
      wo_start(rows_of(g + GA), sem_wo.at[ws], WO_SUB)

    @pl.when(g + GA == NG)
    def _():
      _start_block(w2_hbm, w2_v, sem_w.at[0], W2_SUB)

    m = jnp.max(s, axis=-1, keepdims=True)
    e = jnp.exp(s - m)
    l = jnp.sum(e, axis=-1, keepdims=True)
    p = e.astype(jnp.bfloat16)

    _wait_block(kv_v.at[vs], sem_kv.at[vs])
    r = None
    for j in range(ncb):
      rj = lax.dot_general(p[:, j * 128:(j + 1) * 128], kv_v[vs, j], _NT_DIMS,
                           preferred_element_type=jnp.float32)
      r = rj if r is None else r + rj
    o = jnp.where(diag, r / l, 0.0)

    @pl.when(more)
    def _():
      kv_start(v_hbm, g + GA, vs)

    @pl.when(g + GA == NG)
    def _():
      for (tg, sub), sem in zip(tail, tail_sems):
        wo_start(rows_of(tg), sem, sub)

    @pl.when(g < ni)
    def _():
      acc_s[...] += jnp.dot(o.astype(jnp.bfloat16), wo_v[rows_of(g), :],
                            preferred_element_type=jnp.float32)

    @pl.when(g >= ni)
    def _():
      r_s[jnp.maximum(g - ni, 0)] = o
    return carry

  lax.fori_loop(0, NG, group, 0)

  _wait_block(w2_v, sem_w.at[0])
  b = jnp.dot(h8, w2_v[...], preferred_element_type=jnp.float32)
  out_s[...] = (1.0 - gmix) * b[0:1, :] + gmix * jnp.sum(acc_s[...], axis=0, keepdims=True)
  for i, ((tg, _), sem) in enumerate(zip(tail, tail_sems)):
    _wait_block(wo_v.at[rows_of(tg), :], sem)
    a = jnp.dot(r_s[i].astype(jnp.bfloat16), wo_v[rows_of(tg), :], preferred_element_type=jnp.float32)
    out = out_s[...] + gmix * jnp.sum(a, axis=0, keepdims=True)
    if i + 1 < len(tail):
      out_s[...] = out
  o_ref[...] = out.astype(o_ref.dtype)


@jax.jit
def pallas_gated_mix__sliding_block_cached__glu_gated_swiglu__decode_kernel(
    A_x: jax.Array,
    A_k_cache: jax.Array,
    A_v_cache: jax.Array,
    A_wq: jax.Array,
    A_wo: jax.Array,
    B_x: jax.Array,
    B_w1: jax.Array,
    B_w3: jax.Array,
    B_w2: jax.Array,
    gate_w: jax.Array,
):
  del B_x
  sk = A_k_cache.shape[2]
  win = min(4096, max(256, sk // 4))
  assert A_k_cache.shape == A_v_cache.shape == (1, HQ, sk, DH) and A_x.shape == (1, 1, D)
  assert win % 128 == 0 and sk % 128 == 0

  kt = jnp.swapaxes(A_k_cache, 2, 3).reshape(HD, sk)
  vt = jnp.swapaxes(A_v_cache, 2, 3).reshape(HD, sk)

  any_spec = pl.BlockSpec(memory_space=pl.ANY)
  bf16, f32 = jnp.bfloat16, jnp.float32
  out = pl.pallas_call(
      functools.partial(_kernel, sk=sk, win=win),
      out_shape=jax.ShapeDtypeStruct((1, D), A_x.dtype),
      in_specs=[any_spec] * 9,
      out_specs=pl.BlockSpec(memory_space=pltpu.VMEM),
      scratch_shapes=[
          pltpu.VMEM((1, D), bf16),
          pltpu.VMEM((D // 128, 128), bf16),
          pltpu.VMEM((D, HD), bf16),
          pltpu.VMEM((HD, D), bf16),
          pltpu.VMEM((D, F), bf16),
          pltpu.VMEM((D, F), bf16),
          pltpu.VMEM((F, D), bf16),
          pltpu.VMEM((2 * GA, win // 128, GR, 128), bf16),
          pltpu.VMEM((NG, LROWS, GR), f32),
          pltpu.VMEM((NT, LROWS, GR), f32),
          pltpu.VMEM((LROWS, D), f32),
          pltpu.VMEM((1, D), f32),
          pltpu.SemaphoreType.DMA((2,)),
          pltpu.SemaphoreType.DMA((2 * GA,)),
          pltpu.SemaphoreType.DMA((GA,)),
      ],
      compiler_params=pltpu.CompilerParams(vmem_limit_bytes=100 * 1024 * 1024),
  )(A_x.reshape(1, D), gate_w.reshape(D // 128, 128), kt, vt, A_wq, A_wo, B_w1, B_w3, B_w2)
  return out.reshape(1, 1, D)
```

```python
import functools

import jax
import jax.numpy as jnp
from jax import lax
import jax.experimental.pallas as pl
import jax.experimental.pallas.tpu as pltpu

D = 640
HQ = 32
DH = 192
HD = HQ * DH
F = 1536
G = 2
GR = G * DH
NG = HQ // G
GA = 2
LROWS = 8
NT = 3

KV_SUB = (192, 128)
WQ_SUB = (8, 1024)
W13_SUB = (8, 768)
W2_SUB = (16, 640)
WO_SUB = (48, 640)
WO_TAIL_SUB = (32, 640)
WO_LAST_SUB = (48, 640)

_NT_DIMS = (((1,), (1,)), ((), ()))


def _start_block(src, dst, sem, sub):
  rows, cols = dst.shape
  sr, sc = sub
  assert rows % (2 * sr) == 0 and cols % sc == 0, (dst.shape, sub)
  n = rows // (2 * sr)

  def burst(o):
    for ci in range(cols // sc):
      for h in range(2):
        r = o * sr + h * (rows // 2)
        if not isinstance(r, int):
          r = pl.multiple_of(r, sr)
        pltpu.make_async_copy(src.at[pl.ds(r, sr), pl.ds(ci * sc, sc)],
                              dst.at[pl.ds(r, sr), pl.ds(ci * sc, sc)], sem).start(priority=h)

  if n == 1:
    burst(0)
  else:
    def body(o, carry):
      burst(o)
      return carry
    lax.fori_loop(0, n, body, 0)


def _wait_block(dst, sem):
  pltpu.make_async_copy(dst, dst, sem).wait()


def _kernel(x_hbm, gw_hbm, k_hbm, v_hbm, wq_hbm, wo_hbm, w1_hbm, w3_hbm, w2_hbm,
            o_ref,
            x_v, gw_v, wq_v, wo_v, w1_v, w3_v, w2_v, kv_v, q_s, r_s, acc_s, out_s,
            sem_w, sem_kv, sem_wo, sem_x, *, sk, win):
  col0 = sk - win
  ncb = win // 128
  scale = DH ** -0.5
  ni = NG - NT

  def rows_of(g):
    return pl.ds(g * GR, GR) if isinstance(g, int) else pl.ds(pl.multiple_of(g * GR, GR), GR)

  def kv_start(src, g, slot):
    sr = KV_SUB[0]
    r0 = g * GR if isinstance(g, int) else pl.multiple_of(g * GR, GR)

    def body(cb, carry):
      for i in range(GR // sr):
        pltpu.make_async_copy(
            src.at[pl.ds(r0 + i * sr, sr), pl.ds(pl.multiple_of(col0 + cb * 128, 128), 128)],
            kv_v.at[slot, cb, pl.ds(i * sr, sr), :],
            sem_kv.at[slot]).start(priority=i % 2)
      return carry
    lax.fori_loop(0, ncb, body, 0)

  def wo_start(rows, sem, sub):
    _start_block(wo_hbm.at[rows, :], wo_v.at[rows, :], sem, sub)

  tail_sems = [sem_wo.at[0], sem_wo.at[1], sem_w.at[1]]
  tail = [(g, WO_LAST_SUB if g == NG - 1 else WO_TAIL_SUB) for g in range(ni, NG)]
  assert len(tail) <= len(tail_sems) and NT >= GA

  cp_x = pltpu.make_async_copy(x_hbm, x_v, sem_x.at[0])
  cp_gw = pltpu.make_async_copy(gw_hbm, gw_v, sem_x.at[1])

  _start_block(wq_hbm, wq_v, sem_w.at[0], WQ_SUB)
  cp_x.start()
  cp_gw.start()
  for g in range(GA):
    kv_start(k_hbm, g, 2 * g)
    wo_start(rows_of(g), sem_wo.at[g], WO_SUB)
    kv_start(v_hbm, g, 2 * g + 1)
    if g == 0:
      _start_block(w1_hbm, w1_v, sem_w.at[1], W13_SUB)
      _start_block(w3_hbm, w3_v, sem_w.at[1], W13_SUB)

  _wait_block(wq_v, sem_w.at[0])
  cp_x.wait()
  cp_gw.wait()
  x = x_v[...]
  x8 = jnp.broadcast_to(x, (LROWS, D))
  xf = x.astype(jnp.float32)
  gwf = gw_v[...].astype(jnp.float32)
  prod = xf[:, 0:128] * gwf[0:1, :]
  for r in range(1, D // 128):
    prod = prod + xf[:, r * 128:(r + 1) * 128] * gwf[r:r + 1, :]
  gmix = jax.nn.sigmoid(jnp.sum(prod, axis=-1, keepdims=True))

  row = lax.broadcasted_iota(jnp.int32, (LROWS, GR), 0)
  head_in_group = lax.broadcasted_iota(jnp.int32, (LROWS, GR), 1) // DH
  diag = row == head_in_group

  def q_proj(g, carry):
    qg = jnp.dot(x8, wq_v[:, rows_of(g)], preferred_element_type=jnp.float32)
    q_s[g] = jnp.where(diag, qg.astype(jnp.bfloat16).astype(jnp.float32), 0.0)
    return carry

  lax.fori_loop(0, NG, q_proj, 0)

  _wait_block(w1_v, sem_w.at[1])
  _wait_block(w3_v, sem_w.at[1])
  gate = jnp.dot(x8, w1_v[...], preferred_element_type=jnp.float32)
  up = jnp.dot(x8, w3_v[...], preferred_element_type=jnp.float32)
  gate = gate.astype(jnp.bfloat16).astype(jnp.float32)
  up = up.astype(jnp.bfloat16).astype(jnp.float32)
  h8 = (gate * jax.nn.sigmoid(gate) * up).astype(jnp.bfloat16)

  acc_s[...] = jnp.zeros((LROWS, D), jnp.float32)

  def group(g, carry):
    ks = 2 * lax.rem(g, GA)
    vs = ks + 1
    ws = lax.rem(g, GA)
    more = g + GA < NG
    qb = q_s[g].astype(jnp.bfloat16)
    _wait_block(kv_v.at[ks], sem_kv.at[ks])
    s = jnp.concatenate([jnp.dot(qb, kv_v[ks, j], preferred_element_type=jnp.float32)
                         for j in range(ncb)], axis=1) * scale

    @pl.when(more)
    def _():
      kv_start(k_hbm, g + GA, ks)

    @pl.when(g < ni)
    def _():
      _wait_block(wo_v.at[rows_of(g), :], sem_wo.at[ws])

    @pl.when(g + GA < ni)
    def _():
      wo_start(rows_of(g + GA), sem_wo.at[ws], WO_SUB)

    @pl.when(g + GA == NG)
    def _():
      _start_block(w2_hbm, w2_v, sem_w.at[0], W2_SUB)

    m = jnp.max(s, axis=-1, keepdims=True)
    e = jnp.exp(s - m)
    l = jnp.sum(e, axis=-1, keepdims=True)
    p = e.astype(jnp.bfloat16)

    _wait_block(kv_v.at[vs], sem_kv.at[vs])
    r = None
    for j in range(ncb):
      rj = lax.dot_general(p[:, j * 128:(j + 1) * 128], kv_v[vs, j], _NT_DIMS,
                           preferred_element_type=jnp.float32)
      r = rj if r is None else r + rj
    o = jnp.where(diag, r / l, 0.0)

    @pl.when(more)
    def _():
      kv_start(v_hbm, g + GA, vs)

    @pl.when(g + GA == NG)
    def _():
      for (tg, sub), sem in zip(tail, tail_sems):
        wo_start(rows_of(tg), sem, sub)

    @pl.when(g < ni)
    def _():
      acc_s[...] += jnp.dot(o.astype(jnp.bfloat16), wo_v[rows_of(g), :],
                            preferred_element_type=jnp.float32)

    @pl.when(g >= ni)
    def _():
      r_s[jnp.maximum(g - ni, 0)] = o
    return carry

  lax.fori_loop(0, NG, group, 0)

  _wait_block(w2_v, sem_w.at[0])
  b = jnp.dot(h8, w2_v[...], preferred_element_type=jnp.float32)
  out_s[...] = (1.0 - gmix) * b[0:1, :] + gmix * jnp.sum(acc_s[...], axis=0, keepdims=True)
  for i, ((tg, _), sem) in enumerate(zip(tail, tail_sems)):
    _wait_block(wo_v.at[rows_of(tg), :], sem)
    a = jnp.dot(r_s[i].astype(jnp.bfloat16), wo_v[rows_of(tg), :], preferred_element_type=jnp.float32)
    out = out_s[...] + gmix * jnp.sum(a, axis=0, keepdims=True)
    if i + 1 < len(tail):
      out_s[...] = out
  o_ref[...] = out.astype(o_ref.dtype)


@jax.jit
def pallas_gated_mix__sliding_block_cached__glu_gated_swiglu__decode_kernel(
    A_x: jax.Array,
    A_k_cache: jax.Array,
    A_v_cache: jax.Array,
    A_wq: jax.Array,
    A_wo: jax.Array,
    B_x: jax.Array,
    B_w1: jax.Array,
    B_w3: jax.Array,
    B_w2: jax.Array,
    gate_w: jax.Array,
):
  del B_x
  sk = A_k_cache.shape[2]
  win = min(4096, max(256, sk // 4))
  assert A_k_cache.shape == A_v_cache.shape == (1, HQ, sk, DH) and A_x.shape == (1, 1, D)
  assert win % 128 == 0 and sk % 128 == 0

  kt = jnp.swapaxes(A_k_cache, 2, 3).reshape(HD, sk)
  vt = jnp.swapaxes(A_v_cache, 2, 3).reshape(HD, sk)

  any_spec = pl.BlockSpec(memory_space=pl.ANY)
  bf16, f32 = jnp.bfloat16, jnp.float32
  out = pl.pallas_call(
      functools.partial(_kernel, sk=sk, win=win),
      out_shape=jax.ShapeDtypeStruct((1, D), A_x.dtype),
      in_specs=[any_spec] * 9,
      out_specs=pl.BlockSpec(memory_space=pltpu.VMEM),
      scratch_shapes=[
          pltpu.VMEM((1, D), bf16),
          pltpu.VMEM((D // 128, 128), bf16),
          pltpu.VMEM((D, HD), bf16),
          pltpu.VMEM((HD, D), bf16),
          pltpu.VMEM((D, F), bf16),
          pltpu.VMEM((D, F), bf16),
          pltpu.VMEM((F, D), bf16),
          pltpu.VMEM((2 * GA, win // 128, GR, 128), bf16),
          pltpu.VMEM((NG, LROWS, GR), f32),
          pltpu.VMEM((NT, LROWS, GR), f32),
          pltpu.VMEM((LROWS, D), f32),
          pltpu.VMEM((1, D), f32),
          pltpu.SemaphoreType.DMA((2,)),
          pltpu.SemaphoreType.DMA((2 * GA,)),
          pltpu.SemaphoreType.DMA((GA,)),
          pltpu.SemaphoreType.DMA((2,)),
      ],
      compiler_params=pltpu.CompilerParams(vmem_limit_bytes=100 * 1024 * 1024),
  )(A_x.reshape(1, D), gate_w.reshape(D // 128, 128), kt, vt, A_wq, A_wo, B_w1, B_w3, B_w2)
  return out.reshape(1, 1, D)
```
